```python
import jax
import jax.numpy as jnp

def _softmax(x, axis=-1):
    return jax.nn.softmax(x, axis=axis)
def _gelu(x):
    return jax.nn.gelu(x, approximate=True)
def _silu(x):
    return jax.nn.silu(x)
def _sigmoid(x):
    return jax.nn.sigmoid(x)
def _layernorm(x, axis=-1, eps=1e-5):
    m = jnp.mean(x, axis=axis, keepdims=True)
    v = jnp.var(x, axis=axis, keepdims=True)
    return (x - m) / jnp.sqrt(v + eps)
def _scatter_add(tgt, idx, src, axis=0):
    return tgt.at[idx].add(src)
def _segment_sum(src, seg, n):
    return jax.ops.segment_sum(src, seg, n)
class _Rng:
    def __init__(self, key):
        self._k = key
    def _next(self):
        self._k, sub = jax.random.split(self._k)
        return sub
    def normal(self, shape):
        return jax.random.normal(self._next(), shape, dtype=jnp.bfloat16)
    def randint(self, lo, hi, shape):
        return jax.random.randint(self._next(), shape, lo, hi, dtype=jnp.int32)
    def uniform(self, shape, lo=0.0, hi=1.0):
        return jax.random.uniform(self._next(), shape, jnp.bfloat16, lo, hi)
    def permutation(self, n):
        return jax.random.permutation(self._next(), n)


kernel_name = 'interleave_layers__ssm_conv_s5__ssm_conv_h3__prompt'

def setup_inputs():
    _rng = _Rng(jax.random.key(int.from_bytes(__import__("os").urandom(4), "little")))
    _w = (lambda a: (lambda t: t.astype(jnp.bfloat16) if jnp.issubdtype(t.dtype, jnp.floating) else t)(jnp.asarray(a)))
    def _A_setup():
        B, S, D = 1, 2048, 640
        P = D
        Lambda_re = -0.5 * jnp.exp((lambda *s: _rng.normal(s) * 0.05)(P))
        Lambda_im = (lambda *s: _rng.normal(s) * 0.05)(P) * 1.0
        B_re = (lambda *s: _rng.normal(s) * 0.05)(P, D) * (D ** -0.5)
        B_im = (lambda *s: _rng.normal(s) * 0.05)(P, D) * (D ** -0.5)
        C_re = (lambda *s: _rng.normal(s) * 0.05)(D, P) * (P ** -0.5)
        C_im = (lambda *s: _rng.normal(s) * 0.05)(D, P) * (P ** -0.5)
        log_dt = (lambda *s: _rng.normal(s) * 0.05)(P) * 0.3 - 2.0
        Dskip = (lambda *s: _rng.normal(s) * 0.05)(D)
        return {
            "x": _w((lambda *s: _rng.normal(s) * 0.05)(B, S, D)),
            "Lambda_re": _w(Lambda_re),
            "Lambda_im": _w(Lambda_im),
            "B_re": _w(B_re),
            "B_im": _w(B_im),
            "C_re": _w(C_re),
            "C_im": _w(C_im),
            "log_dt": _w(log_dt),
            "Dskip": _w(Dskip),
        }
    _A_in = _A_setup()

    def _B_setup():
        B, S, D = 1, 2048, 640
        ks = 4
        return {
            "q": _w((lambda *s: _rng.normal(s) * 0.05)(B, S, D)),
            "k": _w((lambda *s: _rng.normal(s) * 0.05)(B, S, D)),
            "v": _w((lambda *s: _rng.normal(s) * 0.05)(B, S, D)),
            "shift_k": _w((lambda *s: _rng.normal(s) * 0.05)(D, ks) * 0.5),
            "ssm_k": _w((lambda *s: _rng.normal(s) * 0.05)(D, S) * (1.0 / S ** 0.5)),
            "ssm_D": _w((lambda *s: _rng.normal(s) * 0.05)(D)),
        }
    _B_in = _B_setup()

    return {
        "A_x": _A_in["x"],
        "A_Lambda_re": _A_in["Lambda_re"],
        "A_Lambda_im": _A_in["Lambda_im"],
        "A_B_re": _A_in["B_re"],
        "A_B_im": _A_in["B_im"],
        "A_C_re": _A_in["C_re"],
        "A_C_im": _A_in["C_im"],
        "A_log_dt": _A_in["log_dt"],
        "A_Dskip": _A_in["Dskip"],
        "B_q": _B_in["q"],
        "B_k": _B_in["k"],
        "B_v": _B_in["v"],
        "B_shift_k": _B_in["shift_k"],
        "B_ssm_k": _B_in["ssm_k"],
        "B_ssm_D": _B_in["ssm_D"],
    }

def reference(A_x, A_Lambda_re, A_Lambda_im, A_B_re, A_B_im, A_C_re, A_C_im, A_log_dt, A_Dskip, B_q, B_k, B_v, B_shift_k, B_ssm_k, B_ssm_D):
    def _A_ref(x, Lambda_re, Lambda_im, B_re, B_im, C_re, C_im, log_dt, Dskip):
        Bsz, L, H = x.shape
        Lam = Lambda_re + 1j * Lambda_im
        Bmat = B_re + 1j * B_im
        Cmat = C_re + 1j * C_im
        dt = jnp.exp(log_dt)
        Lam_bar = jnp.exp(dt * Lam)
        B_bar = ((Lam_bar - 1.0) / Lam)[:, None] * Bmat
        Bu = jnp.einsum("bld,pd->blp", x + 0j, B_bar)
        h = jnp.zeros_like(Bu[:, 0, :])
        hs = []
        for t in range(L):
            h = Lam_bar[None, :] * h + Bu[:, t, :]
            hs.append(h)
        hseq = jnp.stack(hs, 1)
        y = 2.0 * jnp.einsum("blp,dp->bld", hseq, Cmat).real + x * Dskip[None, None, :]
        return y

    def _B_ref(q, k, v, shift_k, ssm_k, ssm_D):
        B, S, D = q.shape
        ks = shift_k.shape[-1]
        k_pad = jnp.pad(k, ((0, 0), (ks - 1, 0), (0, 0)))
        k_shift = jnp.zeros_like(k)
        for t in range(ks):
            k_shift = k_shift + k_pad[:, t:t + S, :] * shift_k[:, ks - 1 - t][None, None, :]
        kv = k_shift * v
        L = 2 * S
        kv_pad = jnp.pad(kv, ((0, 0), (0, S), (0, 0)))
        kf_pad = jnp.pad(ssm_k, ((0, 0), (0, S)))
        kv_f = (lambda x, axes=(-2,-1): jnp.fft.rfft2(x.astype(jnp.float32), axes=axes))(kv_pad[:, None, :, :], axes=(1, 2))
        kf_f = (lambda x, axes=(-2,-1): jnp.fft.rfft2(x.astype(jnp.float32), axes=axes))(kf_pad[:, None, :], axes=(1, 2))
        kf_f = (lambda x, *d: x.transpose(*d))(kf_f, 1, 2, 0)
        y_f = kv_f * kf_f[None, :, :, :]
        y = (lambda x, s, axes=(-2,-1): jnp.fft.irfft2(x, s=s, axes=axes).astype(jnp.bfloat16))(y_f, (1, L), axes=(1, 2))[:, 0, :S, :]
        y = y + kv * ssm_D[None, None, :]
        return q * y

    x = A_x
    x = x + _A_ref(_layernorm(x, axis=-1), A_Lambda_re, A_Lambda_im, A_B_re, A_B_im, A_C_re, A_C_im, A_log_dt, A_Dskip)
    x = x + _B_ref(_layernorm(x, axis=-1), B_k, B_v, B_shift_k, B_ssm_k, B_ssm_D)
    x = x + _A_ref(_layernorm(x, axis=-1), A_Lambda_re, A_Lambda_im, A_B_re, A_B_im, A_C_re, A_C_im, A_log_dt, A_Dskip)
    x = x + _B_ref(_layernorm(x, axis=-1), B_k, B_v, B_shift_k, B_ssm_k, B_ssm_D)
    return x
```

```python
import numpy as np

import jax
import jax.numpy as jnp
from jax import lax
import jax.experimental.pallas as pl
import jax.experimental.pallas.tpu as pltpu

S = 2048
D = 640
LN = 128
NT = D // LN
SEG = 8
J = S // SEG
CH = 32
NCH = J // CH
R = SEG * CH
PW = J // 2 + 4
PF = J + 4
T = 128
NB = S // T
NQ = T // 8
EPS = 1e-5
KPAD = 16


def _dft_constants():
    rho = np.arange(T)
    f = np.concatenate([np.arange(0, T, 2), np.arange(1, T, 2)])
    n = np.arange(T)
    theta = np.pi * np.outer(2 * f + 1, n) / (2 * T)
    c, s = np.cos(theta), -np.sin(theta)
    row_re = 16 * (rho // 8) + rho % 8
    row_im = row_re + 8
    fk = np.zeros((2 * T, T))
    fk[row_re] = c
    fk[row_im] = s
    kappa = np.arange(T)
    g, r = kappa // 16, kappa % 16
    t_of_kappa = np.where(r < 8, 16 * g + 2 * r, 16 * g + 2 * (r - 8) + 1)
    fx = fk[:, t_of_kappa]
    inv = np.zeros((T, 2 * T))
    inv[:, row_re] = c.T / T
    inv[:, row_im] = s.T / T
    bf = jnp.bfloat16
    return fk.astype(bf), fx.astype(bf), inv.astype(bf)


_FK, _FX, _INV = _dft_constants()

_NT_DIMS = (((1,), (1,)), ((), ()))


def _nt(a, b):
    return lax.dot_general(a, b, _NT_DIMS, preferred_element_type=jnp.float32)


def _lo(w):
    return pltpu.bitcast(w << 16, jnp.float32)


def _hi(w):
    return pltpu.bitcast(w & jnp.uint32(0xFFFF0000), jnp.float32)


def _as_bf16(w):
    return pltpu.bitcast(w, jnp.bfloat16)


def _cmul(ar, ai, br, bi):
    return ar * br - ai * bi, ar * bi + ai * br


def _layernorm(x):
    m = jnp.mean(x, axis=-1, keepdims=True)
    d = x - m
    v = jnp.mean(d * d, axis=-1, keepdims=True)
    return d * lax.rsqrt(v + EPS)


def _tile(v, n):
    return v[:, n * LN:(n + 1) * LN]


def _kernel(lre_ref, lim_ref, ldt_ref, dsk_ref, sh_ref, sd_ref, fk_ref, fx_ref, inv_ref,
            x_hbm, bre_hbm, bim_hbm, cre_hbm, cim_hbm, k_hbm, v_hbm, sk_hbm,
            out_hbm,
            xb, bb, cb, kb, vb, skb, cp, xs, gs, ys, gn, wp, hr, hi, ob,
            sems, osem):
    f32 = jnp.float32
    xw = xb.bitcast(jnp.uint32)
    bw = bb.bitcast(jnp.uint32)
    cw = cb.bitcast(jnp.uint32)
    kw = kb.bitcast(jnp.uint32)
    vw = vb.bitcast(jnp.uint32)
    skw = skb.bitcast(jnp.uint32)

    copies = {}
    sem_idx = [0]

    def start(group, src, dst):
        c = pltpu.make_async_copy(src, dst, sems.at[sem_idx[0]])
        sem_idx[0] += 1
        c.start()
        copies.setdefault(group, []).append(c)

    def wait(group):
        for c in copies.pop(group):
            c.wait()

    for n in range(NT):
        col = pl.ds(n * LN, LN)
        for s in range(SEG):
            start("x", x_hbm.at[0, pl.ds(s * J, J), col], xb.at[n, pl.ds(s * 2 * PW, J), :])
    for i, src in enumerate((bre_hbm, bim_hbm)):
        for n in range(NT):
            start("b", src.at[:, pl.ds(n * LN, LN)], bb.at[i, n])
    for i, src in enumerate((cre_hbm, cim_hbm)):
        for n in range(NT):
            start("c", src.at[:, pl.ds(n * LN, LN)], cb.at[i, n])
    for m in range(NB):
        start("sk", sk_hbm.at[:, pl.ds(m * T, T)], skb.at[m])
    for n in range(NT):
        col = pl.ds(n * LN, LN)
        start("kv", k_hbm.at[0, :, col], kb.at[n, pl.ds(KPAD, S), :])
        start("kv", v_hbm.at[0, :, col], vb.at[n])

    def vec(ref):
        return ref[...].astype(f32).reshape(1, D)

    lre, lim = vec(lre_ref), vec(lim_ref)
    dt = jnp.exp(vec(ldt_ref)).astype(jnp.bfloat16).astype(f32)
    ar, ai = dt * lre, dt * lim
    mag = jnp.exp(ar)
    lr1, li1 = mag * jnp.cos(ai), mag * jnp.sin(ai)
    den = lre * lre + lim * lim
    nr = lr1 - 1.0
    sre = (nr * lre + li1 * lim) / den
    sim = (li1 * lre - nr * lim) / den
    lr = jnp.broadcast_to(lr1, (SEG, D))
    li = jnp.broadcast_to(li1, (SEG, D))
    dsk = jnp.broadcast_to(vec(dsk_ref), (R, D))
    pw = [(lr, li)]
    for _ in range(10):
        pr, pi = pw[-1]
        pw.append((pr * pr - pi * pi, 2.0 * pr * pi))
    l2j = J.bit_length() - 1
    seg_pw = [pw[l2j], pw[l2j + 1], pw[l2j + 2]]
    sub = lax.broadcasted_iota(jnp.int32, (SEG, LN), 0)

    def shifted(v, k):
        return jnp.where(sub >= k, pltpu.roll(v, k, 0), 0.0)

    def segment_carry(er, ei, n):
        cr, ci = shifted(er, 1), shifted(ei, 1)
        for k, (ar_, ai_) in zip((1, 2, 4), seg_pw):
            tr, ti = _cmul(_tile(ar_, n), _tile(ai_, n), shifted(cr, k), shifted(ci, k))
            cr, ci = cr + tr, ci + ti
        return cr, ci

    def b_matmul_and_scan(c, u, state):
        ub = u.astype(jnp.bfloat16)
        for n in range(NT):
            rows = pl.ds(n * (LN // 2), LN // 2)
            w = jnp.concatenate(
                [jnp.concatenate([_as_bf16(bw[i, t, rows, :]) for t in range(NT)], axis=1)
                 for i in range(2)], axis=0)
            bu = _nt(ub, w)
            sr, si = state[n]
            l_r, l_i = _tile(lr, n), _tile(li, n)
            for j in range(CH):
                mr, mi = _cmul(l_r, l_i, sr, si)
                sr = mr + bu[8 * j:8 * j + 8, :LN]
                si = mi + bu[8 * j:8 * j + 8, LN:]
                hr[n, pl.ds(c * R + 8 * j, 8), :] = sr
                hi[n, pl.ds(c * R + 8 * j, 8), :] = si
            state[n] = (sr, si)

    def fixup_and_c_matmul(c, carry):
        cols = []
        for n in range(NT):
            cr, ci = carry[n]
            l_r, l_i = _tile(lr, n), _tile(li, n)
            pr, pi = [], []
            for j in range(CH):
                cr, ci = _cmul(l_r, l_i, cr, ci)
                pr.append(hr[n, pl.ds(c * R + 8 * j, 8), :] + cr)
                pi.append(hi[n, pl.ds(c * R + 8 * j, 8), :] + ci)
            carry[n] = (cr, ci)
            cols.append(jnp.concatenate(pr, axis=0).astype(jnp.bfloat16))
            cols.append(jnp.concatenate(pi, axis=0).astype(jnp.bfloat16))
        h = jnp.concatenate(cols, axis=1)
        w = jnp.concatenate([_as_bf16(cp[k]) for k in range(2 * NT)], axis=1)
        return _nt(h, w)

    def load_rows(ref, c):
        return jnp.concatenate([ref[n, pl.ds(c * R, R), :] for n in range(NT)], axis=1)

    def store_rows(ref, c, val):
        for n in range(NT):
            ref[n, pl.ds(c * R, R), :] = _tile(val, n)

    def load_gate(c):
        return jnp.concatenate(
            [jnp.concatenate([gn[n, pl.ds(c * CH + j, SEG, stride=PF), :] for j in range(CH)],
                             axis=0) for n in range(NT)], axis=1)

    def conv_front():
        taps = sh_ref[...].astype(f32)
        sd = jnp.broadcast_to(vec(sd_ref), (8, D))
        fk = fk_ref[...]
        fx = fx_ref[...]
        wait("sk")
        prev = None
        for m in range(NB):
            kf = _nt(fk, _as_bf16(skw[m]))
            for q in range(NQ):
                re, im = kf[16 * q:16 * q + 8], kf[16 * q + 8:16 * q + 16]
                if m == 0:
                    gre, gim = re + sd, im
                else:
                    pre, pim = prev[16 * q:16 * q + 8], prev[16 * q + 8:16 * q + 16]
                    if q < NQ // 2:
                        gre, gim = re - pim, im + pre
                    else:
                        gre, gim = re + pim, im - pre
                for n in range(NT):
                    gs[m * NT + n, 16 * q:16 * q + 8, :] = _tile(gre, n)
                    gs[m * NT + n, 16 * q + 8:16 * q + 16, :] = _tile(gim, n)
            prev = kf
        for n in range(NT):
            kb[n, 0:KPAD, :] = jnp.zeros((KPAD, LN), jnp.bfloat16)
        wait("kv")
        for b in range(NB):
            cols = []
            for n in range(NT):
                a0, a1, a2, a3 = (jnp.broadcast_to(_tile(taps[i:i + 1], n), (T // 2, LN))
                                  for i in range(4))
                base = KPAD // 2 + b * (T // 2)
                w0 = kw[n, pl.ds(base, T // 2), :]
                w1 = kw[n, pl.ds(base - 1, T // 2), :]
                w2 = kw[n, pl.ds(base - 2, T // 2), :]
                k0, k1, k2, k3, k4 = _hi(w0), _lo(w0), _hi(w1), _lo(w1), _hi(w2)
                vv = vw[n, pl.ds(b * (T // 2), T // 2), :]
                even = (a3 * k4 + a2 * k3 + a1 * k2 + a0 * k1) * _lo(vv)
                odd = (a3 * k3 + a2 * k2 + a1 * k1 + a0 * k0) * _hi(vv)
                parts = []
                for g in range(T // 16):
                    parts += [even[8 * g:8 * g + 8], odd[8 * g:8 * g + 8]]
                cols.append(jnp.concatenate(parts, axis=0).astype(jnp.bfloat16))
            xf = jnp.dot(fx, jnp.concatenate(cols, axis=1), preferred_element_type=f32)
            for n in range(NT):
                xs[b * NT + n] = _tile(xf, n)

    def conv_mac():
        for n in range(NT):
            for q in range(NQ):
                re_rows, im_rows = pl.ds(16 * q, 8), pl.ds(16 * q + 8, 8)
                xr = [xs[b * NT + n, re_rows, :] for b in range(NB)]
                xi = [xs[b * NT + n, im_rows, :] for b in range(NB)]
                gr = [gs[b * NT + n, re_rows, :] for b in range(NB)]
                gi = [gs[b * NT + n, im_rows, :] for b in range(NB)]
                for i in range(NB):
                    yr = yi = None
                    for m in range(i + 1):
                        tr, ti = _cmul(gr[m], gi[m], xr[i - m], xi[i - m])
                        yr, yi = (tr, ti) if yr is None else (yr + tr, yi + ti)
                    packed = jnp.concatenate([yr, yi], axis=0).astype(jnp.bfloat16)
                    ys[i * NT + n, pl.ds(8 * q, 8), :] = pltpu.bitcast(packed, jnp.uint32)

    def conv_back():
        inv = inv_ref[...]
        for i in range(NB):
            yv = jnp.concatenate([_as_bf16(ys[i * NT + n]) for n in range(NT)], axis=1)
            y = jnp.dot(inv, yv, preferred_element_type=f32)
            base = (i * T // J) * PF + (i * T) % J
            for n in range(NT):
                gn[n, pl.ds(base, T), :] = _tile(y, n)

    wait("x")
    wait("b")
    zero = jnp.zeros((SEG, LN), f32)
    state = [(zero, zero) for _ in range(NT)]
    for c in range(NCH):
        cols = []
        for n in range(NT):
            parts = []
            for q in range(CH // 2):
                w = xw[n, pl.ds(c * (CH // 2) + q, SEG, stride=PW), :]
                parts += [_lo(w), _hi(w)]
            cols.append(jnp.concatenate(parts, axis=0))
        x0 = jnp.concatenate(cols, axis=1)
        u = _layernorm(x0)
        store_rows(wp, c, x0 + u * dsk)
        b_matmul_and_scan(c, u, state)

    conv_front()
    conv_mac()
    conv_back()

    wait("c")
    s2r, s2i = 2.0 * sre, 2.0 * sim
    for n in range(NT):
        c_re = _as_bf16(cw[0, n]).astype(f32)
        c_im = _as_bf16(cw[1, n]).astype(f32)
        a, b = _tile(s2r, n), _tile(s2i, n)
        cp[2 * n] = pltpu.bitcast((c_re * a - c_im * b).astype(jnp.bfloat16), jnp.uint32)
        cp[2 * n + 1] = pltpu.bitcast((-(c_re * b + c_im * a)).astype(jnp.bfloat16), jnp.uint32)

    carry = [segment_carry(*state[n], n) for n in range(NT)]
    state = [(zero, zero) for _ in range(NT)]
    for c in range(NCH):
        x1 = load_rows(wp, c) + fixup_and_c_matmul(c, carry)
        x2 = x1 + _layernorm(x1) * load_gate(c)
        u = _layernorm(x2)
        store_rows(wp, c, x2 + u * dsk)
        b_matmul_and_scan(c, u, state)

    carry = [segment_carry(*state[n], n) for n in range(NT)]
    outs = []
    for c in range(NCH):
        x3 = load_rows(wp, c) + fixup_and_c_matmul(c, carry)
        x4 = x3 + _layernorm(x3) * load_gate(c)
        for n in range(NT):
            for j in range(CH):
                ob[n, pl.ds(c * CH + j, SEG, stride=PF), :] = x4[8 * j:8 * j + 8, n * LN:(n + 1) * LN]
        for n in range(NT):
            for s in range(SEG):
                cpy = pltpu.make_async_copy(
                    ob.at[n, pl.ds(s * PF + c * CH, CH), :],
                    out_hbm.at[0, pl.ds(s * J + c * CH, CH), pl.ds(n * LN, LN)], osem)
                cpy.start()
                outs.append(cpy)
    for cpy in outs:
        cpy.wait()


@jax.jit
def pallas_interleave_layers__ssm_conv_s5__ssm_conv_h3__prompt_kernel(
    A_x: jax.Array,
    A_Lambda_re: jax.Array,
    A_Lambda_im: jax.Array,
    A_B_re: jax.Array,
    A_B_im: jax.Array,
    A_C_re: jax.Array,
    A_C_im: jax.Array,
    A_log_dt: jax.Array,
    A_Dskip: jax.Array,
    B_q: jax.Array,
    B_k: jax.Array,
    B_v: jax.Array,
    B_shift_k: jax.Array,
    B_ssm_k: jax.Array,
    B_ssm_D: jax.Array,
):
    del B_q
    bf, f32, u32 = jnp.bfloat16, jnp.float32, jnp.uint32
    n_sems = NT * SEG + 2 * NT + 2 * NT + NB + 2 * NT
    vmem = pl.BlockSpec(memory_space=pltpu.VMEM)
    hbm = pl.BlockSpec(memory_space=pl.ANY)
    return pl.pallas_call(
        _kernel,
        out_shape=jax.ShapeDtypeStruct((1, S, D), f32),
        in_specs=[vmem] * 9 + [hbm] * 8,
        out_specs=hbm,
        scratch_shapes=[
            pltpu.VMEM((NT, SEG * 2 * PW, LN), bf),
            pltpu.VMEM((2, NT, D, LN), bf),
            pltpu.VMEM((2, NT, D, LN), bf),
            pltpu.VMEM((NT, KPAD + S, LN), bf),
            pltpu.VMEM((NT, S, LN), bf),
            pltpu.VMEM((NB, D, LN), bf),
            pltpu.VMEM((2 * NT, D // 2, LN), u32),
            pltpu.VMEM((NB * NT, 2 * T, LN), f32),
            pltpu.VMEM((NB * NT, 2 * T, LN), f32),
            pltpu.VMEM((NB * NT, T, LN), u32),
            pltpu.VMEM((NT, SEG * PF, LN), f32),
            pltpu.VMEM((NT, S, LN), f32),
            pltpu.VMEM((NT, S, LN), f32),
            pltpu.VMEM((NT, S, LN), f32),
            pltpu.VMEM((NT, SEG * PF, LN), f32),
            pltpu.SemaphoreType.DMA((n_sems,)),
            pltpu.SemaphoreType.DMA(()),
        ],
        compiler_params=pltpu.CompilerParams(vmem_limit_bytes=112 * 1024 * 1024),
    )(A_Lambda_re, A_Lambda_im, A_log_dt, A_Dskip, B_shift_k.T, B_ssm_D, _FK, _FX, _INV,
      A_x, A_B_re, A_B_im, A_C_re, A_C_im, B_k, B_v, B_ssm_k)
```

```python
import numpy as np

import jax
import jax.numpy as jnp
from jax import lax
import jax.experimental.pallas as pl
import jax.experimental.pallas.tpu as pltpu

def _p(name, default):
    del name
    return default

MODE = _p("MODE", "ABCD")
S = 2048
D = 640
LN = 128
NT = D // LN
SEG = 8
J = S // SEG
CH = 32
NCH = J // CH
R = SEG * CH
PW = J // 2 + 4
PF = J + 4
T = 128
NB = S // T
NQ = T // 8
EPS = 1e-5
KPAD = 16
STRETCH_A = _p("SA", 6.2)
STRETCH_B = _p("SB", 3.3)
GROWS = _p("GROWS", 16)
CH_M1 = _p("CH_M1", 2)
CH_M2 = _p("CH_M2", 4)
CH_E2 = _p("CH_E2", 4)
FIXSER_B = _p("FIXSER_B", 0)
FIXSER_D = _p("FIXSER_D", 0)
NBAR = 6
X4LAST = _p("X4LAST", 1)
MAC_CH = _p("MAC_CH", 1)
MAC_LONG = _p("MAC_LONG", 100)
FULL_D = _p("FULL_D", 1)
D_STEPS = [int(t) for t in _p("DSTEPS", "32,32,32,32,32,32,32,16,8,8").split(",")]
LAST_SPLIT = _p("LAST_SPLIT", 3)
ANCH_G = _p("ANCH_G", 3)
SPLIT_C = _p("SPLIT_C", 0)
CH_G = _p("CH_G", 4)
CH_U = _p("CH_U", 4)
ANCH_D = _p("ANCH_D", 2)
KTICK = _p("KTICK", 1.0)
XTICK = _p("XTICK", 0.0)
CH_HEAD = _p("CH_HEAD", 16)


def _pack_rows(a):
    u = np.asarray(a.astype(jnp.bfloat16)).view(np.uint16).astype(np.uint32)
    return u[0::2] | (u[1::2] << 16)


def _dft_constants():
    rho = np.arange(T)
    f = np.concatenate([np.arange(0, T, 2), np.arange(1, T, 2)])
    n = np.arange(T)
    theta = np.pi * np.outer(2 * f + 1, n) / (2 * T)
    c, s = np.cos(theta), -np.sin(theta)
    row_re = 16 * (rho // 8) + rho % 8
    row_im = row_re + 8
    fk = np.zeros((2 * T, T))
    fk[row_re] = c
    fk[row_im] = s
    kappa = np.arange(T)
    g, r = kappa // 16, kappa % 16
    t_of_kappa = np.where(r < 8, 16 * g + 2 * r, 16 * g + 2 * (r - 8) + 1)
    fx = fk[:, t_of_kappa]
    inv = np.zeros((T, 2 * T))
    inv[:, row_re] = c.T / T
    inv[:, row_im] = s.T / T
    inv = np.concatenate([inv, np.zeros((16, 2 * T))], axis=0)
    return _pack_rows(fk), _pack_rows(fx), _pack_rows(inv)


_FK, _FX, _INV = _dft_constants()

_NT_DIMS = (((1,), (1,)), ((), ()))


def _nt(a, b):
    return lax.dot_general(a, b, _NT_DIMS, preferred_element_type=jnp.float32)


def _nn(a, b):
    return jnp.dot(a, b, preferred_element_type=jnp.float32)


def _lo(w):
    return pltpu.bitcast(w << 16, jnp.float32)


def _hi(w):
    return pltpu.bitcast(w & jnp.uint32(0xFFFF0000), jnp.float32)


def _as_bf16(w):
    return pltpu.bitcast(w, jnp.bfloat16)


def _cmul(ar, ai, br, bi):
    return ar * br - ai * bi, ar * bi + ai * br


def _layernorm(x):
    m = jnp.mean(x, axis=-1, keepdims=True)
    d = x - m
    v = jnp.mean(d * d, axis=-1, keepdims=True)
    return d * lax.rsqrt(v + EPS)


def _tile(v, n):
    return v[:, n * LN:(n + 1) * LN]


def _kernel(lre_hbm, lim_hbm, ldt_hbm, dsk_hbm, sh_hbm, sd_hbm, fk_hbm, fx_hbm, inv_hbm,
            x_hbm, bre_hbm, bim_hbm, cre_hbm, cim_hbm, k_hbm, v_hbm, sk_hbm,
            out_hbm,
            lre_ref, lim_ref, ldt_ref, dsk_ref, sh_ref, sd_ref, fk_ref, fx_ref, inv_ref,
            xb, braw, bw, cb, kb, vb, skb, xs, gs, ys, gn, wp, hr, hi, ob, bar,
            sems, osem):
    f32 = jnp.float32
    bf16 = jnp.bfloat16
    xw = xb.bitcast(jnp.uint32)
    cw = cb.bitcast(jnp.uint32)
    kw = kb.bitcast(jnp.uint32)
    vw = vb.bitcast(jnp.uint32)

    plans, started = {}, {}
    n_sem = [0]

    def plan(group, src, dst):
        plans.setdefault(group, []).append(pltpu.make_async_copy(src, dst, sems.at[n_sem[0]]))
        n_sem[0] += 1

    def start(*groups):
        for g in groups:
            started[g] = plans.pop(g)
            for c in started[g]:
                c.start()

    def wait(*groups):
        for g in groups:
            for c in started.pop(g):
                c.wait()

    for src, dst in ((lre_hbm, lre_ref), (lim_hbm, lim_ref), (ldt_hbm, ldt_ref), (dsk_hbm, dsk_ref),
                     (inv_hbm, inv_ref)):
        plan("par", src, dst)
    for src, dst in ((sh_hbm, sh_ref), (sd_hbm, sd_ref), (fk_hbm, fk_ref), (fx_hbm, fx_ref)):
        plan(("cv", 0), src, dst)
    x_parts = ((0, 3), (3, 6), (6, 8))
    for p, (c0, c1) in enumerate(x_parts):
        for n in range(NT):
            for s in range(SEG):
                plan(("x", p), x_hbm.at[0, pl.ds(s * J + c0 * CH, (c1 - c0) * CH), pl.ds(n * LN, LN)],
                     xb.at[n, pl.ds(s * 2 * PW + c0 * CH, (c1 - c0) * CH), :])
    for n in range(NT):
        for i, src in enumerate((bre_hbm, bim_hbm)):
            plan(("b", 0 if n < 2 else 1), src.at[pl.ds(n * LN, LN), :], braw.at[i, pl.ds(n * LN, LN), :])
        col = pl.ds(n * LN, LN)
        plan(("cv", n), sk_hbm.at[col, :], skb.at[n])
        plan(("cv", n), k_hbm.at[0, :, col], kb.at[n, pl.ds(KPAD, S), :])
        plan(("cv", n), v_hbm.at[0, :, col], vb.at[n])
        for i, src in enumerate((cre_hbm, cim_hbm)):
            plan("c", src.at[:, col], cb.at[i, n])
    for i in range(NBAR):
        plan(("bar", i), bre_hbm.at[pl.ds(0, 16), pl.ds(0, LN)], bar.at[i])
    bar_idx = [0]

    def barrier():
        wait(("bar", bar_idx[0]))
        bar_idx[0] += 1

    start("par", ("x", 0), ("b", 0), ("b", 1))
    for n in range(NT):
        kb[n, 0:KPAD, :] = jnp.zeros((KPAD, LN), bf16)
    wait("par")

    def vec(ref):
        return ref[...].astype(f32).reshape(1, D)

    zmask = inv_ref[T // 2:T // 2 + 8, 0:LN]

    def token_of(v):
        return pltpu.bitcast(pltpu.bitcast(v, jnp.uint32) & zmask, f32)

    def token_of_all(v):
        z = zmask
        for r in range(v.shape[0] // 8):
            for n in range(v.shape[1] // LN):
                z = z & pltpu.bitcast(v[8 * r:8 * r + 8, n * LN:(n + 1) * LN], jnp.uint32)
        return pltpu.bitcast(z, f32)

    lre, lim = vec(lre_ref), vec(lim_ref)
    dt = jnp.exp(vec(ldt_ref)).astype(bf16).astype(f32)
    ar, ai = dt * lre, dt * lim
    mag = jnp.exp(ar)
    lr1, li1 = mag * jnp.cos(ai), mag * jnp.sin(ai)
    den = lre * lre + lim * lim
    nr = lr1 - 1.0
    s2r = 2.0 * ((nr * lre + li1 * lim) / den)
    s2i = 2.0 * ((li1 * lre - nr * lim) / den)
    lr = jnp.broadcast_to(lr1, (SEG, D))
    li = jnp.broadcast_to(-li1, (SEG, D))
    s_cols = [tuple(jnp.broadcast_to(_tile(v, n), (LN, LN)).T for v in (s2r, s2i)) for n in range(NT)]
    dsk = vec(dsk_ref)
    sub = lax.broadcasted_iota(jnp.int32, (SEG, LN), 0)

    def shifted(v, k):
        return jnp.where(sub >= k, pltpu.roll(v, k, 0), 0.0)

    def segment_carry(state):
        pr, pi = lr, li
        for _ in range(J.bit_length() - 1):
            pr, pi = pr * pr - pi * pi, 2.0 * pr * pi
        pws = [(pr, pi)]
        for _ in range(2):
            pr, pi = pr * pr - pi * pi, 2.0 * pr * pi
            pws.append((pr, pi))
        out = []
        for n, (er, ei) in enumerate(state):
            cr, ci = shifted(er, 1), shifted(ei, 1)
            for k, (ar_, ai_) in zip((1, 2, 4), pws):
                tr, ti = _cmul(_tile(ar_, n), _tile(ai_, n), shifted(cr, k), shifted(ci, k))
                cr, ci = cr + tr, ci + ti
            out.append((cr, ci))
        return out

    last_toks = []

    def chained(chains, get_group, body, rows=R, full=False):
        toks = [None] * chains
        res = []
        for g in range(rows // GROWS):
            tiles = get_group(g)
            t = toks[g % chains]
            if t is not None:
                tiles[0] = tiles[0] + jnp.concatenate([t] * (GROWS // 8), axis=0)
            out = body(g, jnp.concatenate(tiles, axis=1))
            toks[g % chains] = token_of_all(out) if full else token_of(out[0:8, 0:LN])
            res.append(out)
        last_toks[:] = [t for t in toks if t is not None]
        return jnp.concatenate(res, axis=0)

    def anchored(words, toks):
        if not toks:
            return words
        z = pltpu.bitcast(toks[0], jnp.uint32)
        for t in toks[1:]:
            z = z | pltpu.bitcast(t, jnp.uint32)
        top = jnp.concatenate([words[0:8, 0:LN] | z, words[0:8, LN:]], axis=1)
        return jnp.concatenate([top, words[8:]], axis=0)

    def b_tile(c, ub, state, n, first=False, toks=None):
        if first:
            a, b = s_cols[n]
            parts = ([], [])
            for r in range(LN // 32):
                rows = pl.ds(n * LN + 32 * r, 32)
                b_re, b_im = braw[0, rows, :].astype(f32), braw[1, rows, :].astype(f32)
                ar_ = jnp.concatenate([a[32 * r:32 * r + 32]] * NT, axis=1)
                bi_ = jnp.concatenate([b[32 * r:32 * r + 32]] * NT, axis=1)
                for i, val in enumerate((b_re * ar_ - b_im * bi_, -(b_re * bi_ + b_im * ar_))):
                    packed = val.astype(bf16)
                    bw[i, pl.ds(n * (LN // 2) + 16 * r, 16), :] = pltpu.bitcast(packed, jnp.uint32)
                    parts[i].append(packed)
            halves = [jnp.concatenate(p, axis=0) for p in parts]
        else:
            halves = [_as_bf16(anchored(bw[i, pl.ds(n * (LN // 2), LN // 2), :], toks if i == 0 else None))
                      for i in range(2)]
        bu = _nt(ub, jnp.concatenate(halves, axis=0))
        sr, si = state[n]
        l_r, l_i = _tile(lr, n), _tile(li, n)
        for j in range(CH):
            mr, mi = _cmul(l_r, l_i, sr, si)
            sr = mr + bu[8 * j:8 * j + 8, :LN]
            si = mi + bu[8 * j:8 * j + 8, LN:]
            hr[n, pl.ds(c * R + 8 * j, 8), :] = sr
            hi[n, pl.ds(c * R + 8 * j, 8), :] = si
        state[n] = (sr, si)

    def fixup(j0, nj, carry, FIXSER=0):
        cols = []
        tok = None
        for n in range(NT):
            cr, ci = carry[n]
            if tok is not None and FIXSER:
                cr = cr + tok
                ci = ci + tok
            l_r, l_i = _tile(lr, n), _tile(li, n)
            pr, pi = [], []
            for j in range(j0, j0 + nj):
                cr, ci = _cmul(l_r, l_i, cr, ci)
                pr.append(hr[n, pl.ds(8 * j, 8), :] + cr)
                pi.append(hi[n, pl.ds(8 * j, 8), :] + ci)
            carry[n] = (cr, ci)
            if FIXSER:
                tok = token_of(cr)
            cols.append(jnp.concatenate(pr, axis=0))
            cols.append(jnp.concatenate(pi, axis=0))
        return jnp.concatenate(cols, axis=1).astype(bf16)

    def c_weights():
        return jnp.concatenate([_as_bf16(cw[k % 2, k // 2]) for k in range(2 * NT)], axis=1)

    def row_group(ref, c, g, r0=None):
        r0 = c * R if r0 is None else r0
        return [ref[n, pl.ds(r0 + g * GROWS, GROWS), :] for n in range(NT)]

    def gate_group(c, g, jbase=None):
        j0 = (c * CH if jbase is None else jbase) + g * GROWS // 8
        return jnp.concatenate(
            [jnp.concatenate([gn[n, pl.ds(j0 + j, SEG, stride=PF), :] for j in range(GROWS // 8)],
                             axis=0) for n in range(NT)], axis=1)

    def store_group(ref, c, g, val):
        for n in range(NT):
            ref[n, pl.ds(c * R + g * GROWS, GROWS), :] = _tile(val, n)

    token = [None] * MAC_CH

    def mac_site(n, i, q):
        re_rows, im_rows = pl.ds(16 * q, 8), pl.ds(16 * q + 8, 8)
        yr = yi = token[q % MAC_CH]
        for m in range(i + 1):
            gr, gi = gs[m * NT + n, re_rows, :], gs[m * NT + n, im_rows, :]
            xr, xi = xs[(i - m) * NT + n, re_rows, :], xs[(i - m) * NT + n, im_rows, :]
            if yr is None:
                yr, yi = _cmul(gr, gi, xr, xi)
            elif m % MAC_LONG == 0:
                yr = (yr + gr * xr) - gi * xi
                yi = (yi + gr * xi) + gi * xr
            else:
                tr, ti = _cmul(gr, gi, xr, xi)
                yr, yi = yr + tr, yi + ti
        ys[i * NT + n, re_rows, :] = yr
        ys[i * NT + n, im_rows, :] = yi
        token[q % MAC_CH] = token_of(yr + yi)

    def conv_block(n, i):
        for q in range(NQ):
            mac_site(n, i, q)
        z = ys[i * NT + n]
        if i > 0:
            zp = ys[(i - 1) * NT + n]
            parts = []
            for q in range(NQ):
                re, im = z[16 * q:16 * q + 8], z[16 * q + 8:16 * q + 16]
                pre, pim = zp[16 * q:16 * q + 8], zp[16 * q + 8:16 * q + 16]
                parts += [re - pim, im + pre] if q < NQ // 2 else [re + pim, im - pre]
            z = jnp.concatenate(parts, axis=0)
        y = _nn(_as_bf16(inv_ref[0:T // 2, :]), z.astype(bf16))
        gn[n, pl.ds((i * T // J) * PF + (i * T) % J, T), :] = y

    pending = []
    credit = [0.0]
    stretch = [STRETCH_A]

    def tick(cycles):
        if not pending:
            credit[0] = 0.0
            return
        credit[0] += cycles
        while pending and credit[0] >= stretch[0] * NQ * (pending[0][1] + 1):
            n, i = pending.pop(0)
            credit[0] -= stretch[0] * NQ * (i + 1) - 64
            conv_block(n, i)

    def drain():
        while pending:
            conv_block(*pending.pop(0))

    def front_k(n):
        sd = jnp.broadcast_to(_tile(vec(sd_ref), n), (8, LN))
        fk = _as_bf16(fk_ref[...])
        for m in range(NB):
            kf = _nt(fk, skb[n, :, pl.ds(m * T, T)])
            if m == 0:
                kf = jnp.concatenate(
                    [kf[8 * r:8 * r + 8] + sd if r % 2 == 0 else kf[8 * r:8 * r + 8]
                     for r in range(2 * NQ)], axis=0)
            gs[m * NT + n] = kf
            tick(64 * KTICK)

    def front_x(n):
        taps = sh_ref[...].astype(f32)
        fx = _as_bf16(fx_ref[...])
        a0, a1, a2, a3 = (jnp.broadcast_to(_tile(taps[i:i + 1], n), (T // 2, LN)) for i in range(4))
        for m in range(NB):
            base = KPAD // 2 + m * (T // 2)
            w0 = kw[n, pl.ds(base, T // 2), :]
            w1 = kw[n, pl.ds(base - 1, T // 2), :]
            w2 = kw[n, pl.ds(base - 2, T // 2), :]
            k0, k1, k2, k3, k4 = _hi(w0), _lo(w0), _hi(w1), _lo(w1), _hi(w2)
            vv = vw[n, pl.ds(m * (T // 2), T // 2), :]
            even = (a3 * k4 + a2 * k3 + a1 * k2 + a0 * k1) * _lo(vv)
            odd = (a3 * k3 + a2 * k2 + a1 * k1 + a0 * k0) * _hi(vv)
            parts = []
            for g in range(T // 16):
                parts += [even[8 * g:8 * g + 8], odd[8 * g:8 * g + 8]]
            xs[m * NT + n] = _nn(fx, jnp.concatenate(parts, axis=0).astype(bf16))
            tick(64 * XTICK)
        for i in range(NB):
            pending.append((n, i))

    zero = jnp.zeros((SEG, LN), f32)
    state = [(zero, zero) for _ in range(NT)]

    def m1_prep(c, chains):
        def get(g):
            tiles = []
            for n in range(NT):
                parts = []
                for q in range(GROWS // 16):
                    w = xw[n, pl.ds(c * (CH // 2) + g * (GROWS // 16) + q, SEG, stride=PW), :]
                    parts += [_lo(w), _hi(w)]
                tiles.append(jnp.concatenate(parts, axis=0))
            return tiles

        def body(g, x0):
            u = _layernorm(x0)
            store_group(wp, c, g, x0 + u * dsk)
            return u
        return chained(chains, get, body).astype(bf16)

    def m_tiles(c, ub, tiles, first=False, toks=None, at=None):
        for n in tiles:
            b_tile(c, ub, state, n, first, toks if n == at else None)
            tick(640)


    doA = "A" in MODE
    ub = {}

    def prep(c, chains=None):
        if doA:
            ub[c] = m1_prep(c, chains or CH_M1)

    def mm(c, tiles=range(NT), first=False):
        if doA:
            m_tiles(c, ub[c], tiles, first)

    def fk_(n):
        if doA:
            front_k(n)

    def fx_(n):
        if doA:
            front_x(n)

    wait(("x", 0), ("b", 0))
    start(("cv", 0))
    prep(0, CH_HEAD)
    mm(0, range(0, 2), True)
    wait(("b", 1))
    start(("x", 1))
    prep(1)
    mm(0, range(2, NT), True)
    prep(2)
    mm(1)
    wait(("cv", 0), ("x", 1))
    start(("cv", 1), ("cv", 2))
    fk_(0); prep(3); mm(2); fx_(0)
    wait(("cv", 1))
    start(("x", 2))
    fk_(1); prep(4); mm(3); fx_(1)
    wait(("cv", 2), ("x", 2))
    start(("cv", 3), "c")
    fk_(2); prep(5); mm(4); fx_(2)
    wait(("cv", 3))
    start(("cv", 4), *[("bar", i) for i in range(NBAR)])
    fk_(3); prep(6); mm(5); prep(7); mm(6); fx_(3)
    wait(("cv", 4))
    fk_(4)
    if X4LAST:
        mm(7); fx_(4)
    else:
        fx_(4); held = pending[-NB:]; del pending[-NB:]; mm(7); pending.extend(held)
    wait("c")
    if doA:
        pass
    elif "B" in MODE:
        for n in range(NT):
            for i in range(NB):
                pending.append((n, i))
        for _ in range(_p("SKIP", 44)):
            pending.pop(0)

    stretch[0] = STRETCH_B
    if "B" in MODE:
        carry = segment_carry(state)
        for c in range(NCH):
            y = _nt(fixup(c * CH, CH, carry, FIXSER_B), c_weights())
            for n in range(NT):
                wp[n, pl.ds(c * R, R), :] = wp[n, pl.ds(c * R, R), :] + _tile(y, n)
            tick(3200)
        drain()
    barrier()

    state[:] = [(zero, zero) for _ in range(NT)]
    if "C" in MODE and SPLIT_C:
        def stage_g(c, chains):
            def body(g, x1):
                x2 = x1 + _layernorm(x1) * gate_group(c, g)
                store_group(wp, c, g, x2)
                return x2
            chained(chains, lambda g: row_group(wp, c, g), body)

        def stage_u(c, chains):
            def body(g, x2):
                u = _layernorm(x2)
                store_group(wp, c, g, x2 + u * dsk)
                return u
            return chained(chains, lambda g: row_group(wp, c, g), body).astype(bf16)

        stage_g(0, CH_HEAD)
        nxt = stage_u(0, CH_HEAD)
        stage_g(1, CH_HEAD)
        for c in range(NCH):
            cur = nxt
            toks = None
            if c + 2 < NCH:
                stage_g(c + 2, CH_G)
                toks = list(last_toks)
            if c + 1 < NCH:
                nxt = stage_u(c + 1, CH_U)
            m_tiles(c, cur, range(NT), toks=toks, at=ANCH_G)
    elif "C" in MODE:
        for c in range(NCH):
            def body(g, x1):
                x2 = x1 + _layernorm(x1) * gate_group(c, g)
                u = _layernorm(x2)
                store_group(wp, c, g, x2 + u * dsk)
                return u
            ub2 = chained(CH_HEAD if c == 0 else CH_M2, lambda g: row_group(wp, c, g), body).astype(bf16)
            m_tiles(c, ub2, range(NT))
    barrier()

    outs = []
    if "D" in MODE:
        carry = segment_carry(state)
        anchors = {}
        j0 = 0
        for c, nj in enumerate(D_STEPS):
            for k, t in enumerate(anchors.pop(c - ANCH_D, [])):
                carry[k % NT] = (carry[k % NT][0] + t, carry[k % NT][1])
            y = _nt(fixup(j0, nj, carry, FIXSER_D), c_weights())

            def get(g):
                return [t + y[g * GROWS:(g + 1) * GROWS, n * LN:(n + 1) * LN]
                        for n, t in enumerate(row_group(wp, 0, g, 8 * j0))]

            def body(g, x3):
                x4 = x3 + _layernorm(x3) * gate_group(0, g, j0)
                for n in range(NT):
                    for j in range(GROWS // 8):
                        ob[n, pl.ds(j0 + g * GROWS // 8 + j, SEG, stride=PF), :] = (
                            x4[8 * j:8 * j + 8, n * LN:(n + 1) * LN])
                return x4
            chained(CH_E2 if c + ANCH_D < len(D_STEPS) else CH_HEAD, get, body, 8 * nj, bool(FULL_D))
            anchors[c] = list(last_toks)
            for n in range(NT):
                for s in range(SEG):
                    cpy = pltpu.make_async_copy(
                        ob.at[n, pl.ds(s * PF + j0, nj), :],
                        out_hbm.at[0, pl.ds(s * J + j0, nj), pl.ds(n * LN, LN)], osem)
                    cpy.start()
                    outs.append(cpy)
            j0 += nj
        assert j0 == J
    while bar_idx[0] < NBAR:
        barrier()
    if MODE != "ABCD":
        for buf in (wp, hr, hi):
            pltpu.make_async_copy(buf.at[0], out_hbm.at[0, :, pl.ds(0, LN)], osem).start()
            pltpu.make_async_copy(buf.at[0], out_hbm.at[0, :, pl.ds(0, LN)], osem).wait()
        for buf in (gn,):
            pltpu.make_async_copy(buf.at[0, pl.ds(0, S)], out_hbm.at[0, :, pl.ds(0, LN)], osem).start()
            pltpu.make_async_copy(buf.at[0, pl.ds(0, S)], out_hbm.at[0, :, pl.ds(0, LN)], osem).wait()
        for buf in (xs, gs):
            pltpu.make_async_copy(buf.at[0], out_hbm.at[0, pl.ds(0, 256), pl.ds(0, LN)], osem).start()
            pltpu.make_async_copy(buf.at[0], out_hbm.at[0, pl.ds(0, 256), pl.ds(0, LN)], osem).wait()
    assert not plans and not started, (plans.keys(), started.keys())
    for cpy in outs:
        cpy.wait()


@jax.jit
def pallas_interleave_layers__ssm_conv_s5__ssm_conv_h3__prompt_kernel(
    A_x: jax.Array,
    A_Lambda_re: jax.Array,
    A_Lambda_im: jax.Array,
    A_B_re: jax.Array,
    A_B_im: jax.Array,
    A_C_re: jax.Array,
    A_C_im: jax.Array,
    A_log_dt: jax.Array,
    A_Dskip: jax.Array,
    B_q: jax.Array,
    B_k: jax.Array,
    B_v: jax.Array,
    B_shift_k: jax.Array,
    B_ssm_k: jax.Array,
    B_ssm_D: jax.Array,
):
    del B_q
    bf, f32, u32 = jnp.bfloat16, jnp.float32, jnp.uint32
    n_sems = 9 + 3 * NT * SEG + 2 * NT + 3 * NT + 2 * NT + NBAR
    hbm = pl.BlockSpec(memory_space=pl.ANY)
    return pl.pallas_call(
        _kernel,
        out_shape=jax.ShapeDtypeStruct((1, S, D), f32),
        in_specs=[hbm] * 17,
        out_specs=hbm,
        scratch_shapes=[
            pltpu.VMEM((D,), bf), pltpu.VMEM((D,), bf), pltpu.VMEM((D,), bf), pltpu.VMEM((D,), bf),
            pltpu.VMEM((4, D), bf), pltpu.VMEM((D,), bf),
            pltpu.VMEM((T, T), u32), pltpu.VMEM((T, T), u32), pltpu.VMEM((T // 2 + 8, 2 * T), u32),
            pltpu.VMEM((NT, SEG * 2 * PW, LN), bf),
            pltpu.VMEM((2, D, D), bf),
            pltpu.VMEM((2, D // 2, D), u32),
            pltpu.VMEM((2, NT, D, LN), bf),
            pltpu.VMEM((NT, KPAD + S, LN), bf),
            pltpu.VMEM((NT, S, LN), bf),
            pltpu.VMEM((NT, LN, S), bf),
            pltpu.VMEM((NB * NT, 2 * T, LN), f32),
            pltpu.VMEM((NB * NT, 2 * T, LN), f32),
            pltpu.VMEM((NB * NT, 2 * T, LN), f32),
            pltpu.VMEM((NT, SEG * PF, LN), f32),
            pltpu.VMEM((NT, S, LN), f32),
            pltpu.VMEM((NT, S, LN), f32),
            pltpu.VMEM((NT, S, LN), f32),
            pltpu.VMEM((NT, SEG * PF, LN), f32),
            pltpu.VMEM((NBAR, 16, LN), bf),
            pltpu.SemaphoreType.DMA((n_sems,)),
            pltpu.SemaphoreType.DMA(()),
        ],
        compiler_params=pltpu.CompilerParams(vmem_limit_bytes=112 * 1024 * 1024),
    )(A_Lambda_re, A_Lambda_im, A_log_dt, A_Dskip, B_shift_k.T, B_ssm_D, _FK, _FX, _INV,
      A_x, A_B_re, A_B_im, A_C_re, A_C_im, B_k, B_v, B_ssm_k)
```

```python
import numpy as np

import jax
import jax.numpy as jnp
from jax import lax
import jax.experimental.pallas as pl
import jax.experimental.pallas.tpu as pltpu

def _p(name, default):
    del name
    return default

MODE = _p("MODE", "ABCD")
S = 2048
D = 640
LN = 128
NT = D // LN
SEG = 8
J = S // SEG
CH = 32
NCH = J // CH
R = SEG * CH
PW = J // 2 + 4
PF = J + 4
T = 128
NB = S // T
NQ = T // 8
EPS = 1e-5
X_PARTS = ((0, 104), (104, 144), (144, 216), (216, 256))
KPAD = 16
STRETCH_A = _p("SA", 6.2)
STRETCH_B = _p("SB", 3.3)
GROWS = _p("GROWS", 16)
CH_M1 = _p("CH_M1", 2)
CH_M2 = _p("CH_M2", 4)
CH_E2 = _p("CH_E2", 4)
FIXSER_B = _p("FIXSER_B", 0)
FIXSER_D = _p("FIXSER_D", 0)
NBAR = 6
MERGE_BC = _p("MERGE_BC", 0)
CH_C0 = _p("CH_C0", 16)
X4LAST = _p("X4LAST", 1)
MAC_CH = _p("MAC_CH", 1)
MAC_LONG = _p("MAC_LONG", 100)
FULL_D = _p("FULL_D", 1)
D_STEPS = [int(t) for t in _p("DSTEPS", "32,32,32,32,32,32,32,16,8,8").split(",")]
LAST_SPLIT = _p("LAST_SPLIT", 3)
ANCH_G = _p("ANCH_G", 3)
SPLIT_C = _p("SPLIT_C", 0)
CH_G = _p("CH_G", 4)
CH_U = _p("CH_U", 4)
ANCH_D = _p("ANCH_D", 2)
KTICK = _p("KTICK", 1.0)
XTICK = _p("XTICK", 0.0)
CH_HEAD = _p("CH_HEAD", 16)


def _pack_rows(a):
    u = np.asarray(a.astype(jnp.bfloat16)).view(np.uint16).astype(np.uint32)
    return u[0::2] | (u[1::2] << 16)


def _dft_constants():
    rho = np.arange(T)
    f = np.concatenate([np.arange(0, T, 2), np.arange(1, T, 2)])
    n = np.arange(T)
    theta = np.pi * np.outer(2 * f + 1, n) / (2 * T)
    c, s = np.cos(theta), -np.sin(theta)
    row_re = 16 * (rho // 8) + rho % 8
    row_im = row_re + 8
    fk = np.zeros((2 * T, T))
    fk[row_re] = c
    fk[row_im] = s
    kappa = np.arange(T)
    g, r = kappa // 16, kappa % 16
    t_of_kappa = np.where(r < 8, 16 * g + 2 * r, 16 * g + 2 * (r - 8) + 1)
    fx = fk[:, t_of_kappa]
    inv = np.zeros((T, 2 * T))
    inv[:, row_re] = c.T / T
    inv[:, row_im] = s.T / T
    inv = np.concatenate([inv, np.zeros((16, 2 * T))], axis=0)
    return _pack_rows(fk), _pack_rows(fx), _pack_rows(inv)


_FK, _FX, _INV = _dft_constants()

_NT_DIMS = (((1,), (1,)), ((), ()))


def _nt(a, b):
    return lax.dot_general(a, b, _NT_DIMS, preferred_element_type=jnp.float32)


def _nn(a, b):
    return jnp.dot(a, b, preferred_element_type=jnp.float32)


def _lo(w):
    return pltpu.bitcast(w << 16, jnp.float32)


def _hi(w):
    return pltpu.bitcast(w & jnp.uint32(0xFFFF0000), jnp.float32)


def _as_bf16(w):
    return pltpu.bitcast(w, jnp.bfloat16)


def _cmul(ar, ai, br, bi):
    return ar * br - ai * bi, ar * bi + ai * br


def _layernorm(x):
    m = jnp.mean(x, axis=-1, keepdims=True)
    d = x - m
    v = jnp.mean(d * d, axis=-1, keepdims=True)
    return d * lax.rsqrt(v + EPS)


def _tile(v, n):
    return v[:, n * LN:(n + 1) * LN]


def _kernel(lre_hbm, lim_hbm, ldt_hbm, dsk_hbm, sh_hbm, sd_hbm, fk_hbm, fx_hbm, inv_hbm,
            x_hbm, bre_hbm, bim_hbm, cre_hbm, cim_hbm, k_hbm, v_hbm, sk_hbm,
            out_hbm,
            lre_ref, lim_ref, ldt_ref, dsk_ref, sh_ref, sd_ref, fk_ref, fx_ref, inv_ref,
            xb0, xb1, xb2, xb3, braw, bw, cb, kb, vb, skb, xs, gs, ys, gn, wp, hr, hi, ob, bar,
            sems, osem):
    f32 = jnp.float32
    bf16 = jnp.bfloat16
    xbs = (xb0, xb1, xb2, xb3)
    xws = [b.bitcast(jnp.uint32) for b in xbs]
    cw = cb.bitcast(jnp.uint32)
    kw = kb.bitcast(jnp.uint32)
    vw = vb.bitcast(jnp.uint32)

    plans, started = {}, {}

    sem_of = {}

    def plan(group, src, dst):
        sem = sem_of.setdefault(group, len(sem_of))
        plans.setdefault(group, []).append(pltpu.make_async_copy(src, dst, sems.at[sem]))

    def start(*groups):
        for g in groups:
            started[g] = plans.pop(g)
            for c in started[g]:
                c.start()

    def wait(*groups):
        for g in groups:
            copies = started.pop(g)
            if g in fills:
                pltpu.make_async_copy(fills[g], fills[g], sems.at[sem_of[g]]).wait()
            else:
                for c in copies:
                    c.wait()

    for src, dst in ((lre_hbm, lre_ref), (lim_hbm, lim_ref), (ldt_hbm, ldt_ref), (dsk_hbm, dsk_ref),
                     (inv_hbm, inv_ref)):
        plan("par", src, dst)
    for src, dst in ((sh_hbm, sh_ref), (sd_hbm, sd_ref), (fk_hbm, fk_ref), (fx_hbm, fx_ref)):
        plan(("cv", 0), src, dst)
    fills = {}
    for p, (r0, r1) in enumerate(X_PARTS):
        fills["x", p] = xbs[p]
        for n in range(NT):
            for s in range(SEG):
                plan(("x", p), x_hbm.at[0, pl.ds(s * J + r0, r1 - r0), pl.ds(n * LN, LN)],
                     xbs[p].at[n, pl.ds(s * (r1 - r0), r1 - r0), :])
    fills["c"] = cb
    for n in range(NT):
        for i, src in enumerate((bre_hbm, bim_hbm)):
            plan(("b", 0 if n < 2 else 1), src.at[pl.ds(n * LN, LN), :], braw.at[i, pl.ds(n * LN, LN), :])
        col = pl.ds(n * LN, LN)
        plan(("cv", n), sk_hbm.at[col, :], skb.at[n])
        plan(("cv", n), k_hbm.at[0, :, col], kb.at[n, pl.ds(KPAD, S), :])
        plan(("cv", n), v_hbm.at[0, :, col], vb.at[n])
        for i, src in enumerate((cre_hbm, cim_hbm)):
            plan("c", src.at[:, col], cb.at[i, n])
    for i in range(NBAR):
        plan(("bar", i), bre_hbm.at[pl.ds(0, 16), pl.ds(0, LN)], bar.at[i])
    bar_idx = [0]

    def barrier():
        wait(("bar", bar_idx[0]))
        bar_idx[0] += 1

    start("par", ("x", 0), ("b", 0), ("b", 1))
    for n in range(NT):
        kb[n, 0:KPAD, :] = jnp.zeros((KPAD, LN), bf16)
    wait("par")

    def vec(ref):
        return ref[...].astype(f32).reshape(1, D)

    zmask = inv_ref[T // 2:T // 2 + 8, 0:LN]

    def token_of(v):
        return pltpu.bitcast(pltpu.bitcast(v, jnp.uint32) & zmask, f32)

    def token_of_all(v):
        z = zmask
        for r in range(v.shape[0] // 8):
            for n in range(v.shape[1] // LN):
                z = z & pltpu.bitcast(v[8 * r:8 * r + 8, n * LN:(n + 1) * LN], jnp.uint32)
        return pltpu.bitcast(z, f32)

    lre, lim = vec(lre_ref), vec(lim_ref)
    dt = jnp.exp(vec(ldt_ref)).astype(bf16).astype(f32)
    ar, ai = dt * lre, dt * lim
    mag = jnp.exp(ar)
    lr1, li1 = mag * jnp.cos(ai), mag * jnp.sin(ai)
    den = lre * lre + lim * lim
    nr = lr1 - 1.0
    s2r = 2.0 * ((nr * lre + li1 * lim) / den)
    s2i = 2.0 * ((li1 * lre - nr * lim) / den)
    lr = jnp.broadcast_to(lr1, (SEG, D))
    li = jnp.broadcast_to(-li1, (SEG, D))
    s_cols = [tuple(jnp.broadcast_to(_tile(v, n), (LN, LN)).T for v in (s2r, s2i)) for n in range(NT)]
    dsk = vec(dsk_ref)
    sub = lax.broadcasted_iota(jnp.int32, (SEG, LN), 0)

    def shifted(v, k):
        return jnp.where(sub >= k, pltpu.roll(v, k, 0), 0.0)

    def segment_carry(state):
        pr, pi = lr, li
        for _ in range(J.bit_length() - 1):
            pr, pi = pr * pr - pi * pi, 2.0 * pr * pi
        pws = [(pr, pi)]
        for _ in range(2):
            pr, pi = pr * pr - pi * pi, 2.0 * pr * pi
            pws.append((pr, pi))
        out = []
        for n, (er, ei) in enumerate(state):
            cr, ci = shifted(er, 1), shifted(ei, 1)
            for k, (ar_, ai_) in zip((1, 2, 4), pws):
                tr, ti = _cmul(_tile(ar_, n), _tile(ai_, n), shifted(cr, k), shifted(ci, k))
                cr, ci = cr + tr, ci + ti
            out.append((cr, ci))
        return out

    last_toks = []

    def chained(chains, get_group, body, rows=R, full=False):
        toks = [None] * chains
        res = []
        for g in range(rows // GROWS):
            tiles = get_group(g)
            t = toks[g % chains]
            if t is not None:
                tiles[0] = tiles[0] + jnp.concatenate([t] * (GROWS // 8), axis=0)
            out = body(g, jnp.concatenate(tiles, axis=1))
            toks[g % chains] = token_of_all(out) if full else token_of(out[0:8, 0:LN])
            res.append(out)
        last_toks[:] = [t for t in toks if t is not None]
        return jnp.concatenate(res, axis=0)

    def anchored(words, toks):
        if not toks:
            return words
        z = pltpu.bitcast(toks[0], jnp.uint32)
        for t in toks[1:]:
            z = z | pltpu.bitcast(t, jnp.uint32)
        top = jnp.concatenate([words[0:8, 0:LN] | z, words[0:8, LN:]], axis=1)
        return jnp.concatenate([top, words[8:]], axis=0)

    def b_tile(c, ub, state, n, first=False, toks=None):
        if first:
            a, b = s_cols[n]
            parts = ([], [])
            for r in range(LN // 32):
                rows = pl.ds(n * LN + 32 * r, 32)
                b_re, b_im = braw[0, rows, :].astype(f32), braw[1, rows, :].astype(f32)
                ar_ = jnp.concatenate([a[32 * r:32 * r + 32]] * NT, axis=1)
                bi_ = jnp.concatenate([b[32 * r:32 * r + 32]] * NT, axis=1)
                for i, val in enumerate((b_re * ar_ - b_im * bi_, -(b_re * bi_ + b_im * ar_))):
                    packed = val.astype(bf16)
                    bw[i, pl.ds(n * (LN // 2) + 16 * r, 16), :] = pltpu.bitcast(packed, jnp.uint32)
                    parts[i].append(packed)
            halves = [jnp.concatenate(p, axis=0) for p in parts]
        else:
            halves = [_as_bf16(anchored(bw[i, pl.ds(n * (LN // 2), LN // 2), :], toks if i == 0 else None))
                      for i in range(2)]
        bu = _nt(ub, jnp.concatenate(halves, axis=0))
        sr, si = state[n]
        l_r, l_i = _tile(lr, n), _tile(li, n)
        for j in range(CH):
            mr, mi = _cmul(l_r, l_i, sr, si)
            sr = mr + bu[8 * j:8 * j + 8, :LN]
            si = mi + bu[8 * j:8 * j + 8, LN:]
            hr[n, pl.ds(c * R + 8 * j, 8), :] = sr
            hi[n, pl.ds(c * R + 8 * j, 8), :] = si
        state[n] = (sr, si)

    def fixup(j0, nj, carry, FIXSER=0):
        cols = []
        tok = None
        for n in range(NT):
            cr, ci = carry[n]
            if tok is not None and FIXSER:
                cr = cr + tok
                ci = ci + tok
            l_r, l_i = _tile(lr, n), _tile(li, n)
            pr, pi = [], []
            for j in range(j0, j0 + nj):
                cr, ci = _cmul(l_r, l_i, cr, ci)
                pr.append(hr[n, pl.ds(8 * j, 8), :] + cr)
                pi.append(hi[n, pl.ds(8 * j, 8), :] + ci)
            carry[n] = (cr, ci)
            if FIXSER:
                tok = token_of(cr)
            cols.append(jnp.concatenate(pr, axis=0))
            cols.append(jnp.concatenate(pi, axis=0))
        return jnp.concatenate(cols, axis=1).astype(bf16)

    def c_weights():
        return jnp.concatenate([_as_bf16(cw[k % 2, k // 2]) for k in range(2 * NT)], axis=1)

    def row_group(ref, c, g, r0=None):
        r0 = c * R if r0 is None else r0
        return [ref[n, pl.ds(r0 + g * GROWS, GROWS), :] for n in range(NT)]

    def gate_group(c, g, jbase=None):
        j0 = (c * CH if jbase is None else jbase) + g * GROWS // 8
        return jnp.concatenate(
            [jnp.concatenate([gn[n, pl.ds(j0 + j, SEG, stride=PF), :] for j in range(GROWS // 8)],
                             axis=0) for n in range(NT)], axis=1)

    def store_group(ref, c, g, val):
        for n in range(NT):
            ref[n, pl.ds(c * R + g * GROWS, GROWS), :] = _tile(val, n)

    token = [None] * MAC_CH

    def mac_site(n, i, q):
        re_rows, im_rows = pl.ds(16 * q, 8), pl.ds(16 * q + 8, 8)
        yr = yi = token[q % MAC_CH]
        for m in range(i + 1):
            gr, gi = gs[m * NT + n, re_rows, :], gs[m * NT + n, im_rows, :]
            xr, xi = xs[(i - m) * NT + n, re_rows, :], xs[(i - m) * NT + n, im_rows, :]
            if yr is None:
                yr, yi = _cmul(gr, gi, xr, xi)
            elif m % MAC_LONG == 0:
                yr = (yr + gr * xr) - gi * xi
                yi = (yi + gr * xi) + gi * xr
            else:
                tr, ti = _cmul(gr, gi, xr, xi)
                yr, yi = yr + tr, yi + ti
        ys[i * NT + n, re_rows, :] = yr
        ys[i * NT + n, im_rows, :] = yi
        token[q % MAC_CH] = token_of(yr + yi)

    def conv_block(n, i):
        for q in range(NQ):
            mac_site(n, i, q)
        z = ys[i * NT + n]
        if i > 0:
            zp = ys[(i - 1) * NT + n]
            parts = []
            for q in range(NQ):
                re, im = z[16 * q:16 * q + 8], z[16 * q + 8:16 * q + 16]
                pre, pim = zp[16 * q:16 * q + 8], zp[16 * q + 8:16 * q + 16]
                parts += [re - pim, im + pre] if q < NQ // 2 else [re + pim, im - pre]
            z = jnp.concatenate(parts, axis=0)
        y = _nn(_as_bf16(inv_ref[0:T // 2, :]), z.astype(bf16))
        gn[n, pl.ds((i * T // J) * PF + (i * T) % J, T), :] = y

    pending = []
    credit = [0.0]
    stretch = [STRETCH_A]

    def tick(cycles):
        if not pending:
            credit[0] = 0.0
            return
        credit[0] += cycles
        while pending and credit[0] >= stretch[0] * NQ * (pending[0][1] + 1):
            n, i = pending.pop(0)
            credit[0] -= stretch[0] * NQ * (i + 1) - 64
            conv_block(n, i)

    def drain():
        while pending:
            conv_block(*pending.pop(0))

    def front_k(n):
        sd = jnp.broadcast_to(_tile(vec(sd_ref), n), (8, LN))
        fk = _as_bf16(fk_ref[...])
        for m in range(NB):
            kf = _nt(fk, skb[n, :, pl.ds(m * T, T)])
            if m == 0:
                kf = jnp.concatenate(
                    [kf[8 * r:8 * r + 8] + sd if r % 2 == 0 else kf[8 * r:8 * r + 8]
                     for r in range(2 * NQ)], axis=0)
            gs[m * NT + n] = kf
            tick(64 * KTICK)

    def front_x(n):
        taps = sh_ref[...].astype(f32)
        fx = _as_bf16(fx_ref[...])
        a0, a1, a2, a3 = (jnp.broadcast_to(_tile(taps[i:i + 1], n), (T // 2, LN)) for i in range(4))
        for m in range(NB):
            base = KPAD // 2 + m * (T // 2)
            w0 = kw[n, pl.ds(base, T // 2), :]
            w1 = kw[n, pl.ds(base - 1, T // 2), :]
            w2 = kw[n, pl.ds(base - 2, T // 2), :]
            k0, k1, k2, k3, k4 = _hi(w0), _lo(w0), _hi(w1), _lo(w1), _hi(w2)
            vv = vw[n, pl.ds(m * (T // 2), T // 2), :]
            even = (a3 * k4 + a2 * k3 + a1 * k2 + a0 * k1) * _lo(vv)
            odd = (a3 * k3 + a2 * k2 + a1 * k1 + a0 * k0) * _hi(vv)
            parts = []
            for g in range(T // 16):
                parts += [even[8 * g:8 * g + 8], odd[8 * g:8 * g + 8]]
            xs[m * NT + n] = _nn(fx, jnp.concatenate(parts, axis=0).astype(bf16))
            tick(64 * XTICK)
        for i in range(NB):
            pending.append((n, i))

    zero = jnp.zeros((SEG, LN), f32)
    state = [(zero, zero) for _ in range(NT)]

    def m1_prep(c, chains):
        def get(g):
            tiles = []
            for n in range(NT):
                parts = []
                for q in range(GROWS // 16):
                    row = c * CH + g * GROWS // 8 + 2 * q
                    p = max(i for i, (r0, _) in enumerate(X_PARTS) if r0 <= row)
                    r0, r1 = X_PARTS[p]
                    w = xws[p][n, pl.ds((row - r0) // 2, SEG, stride=(r1 - r0) // 2), :]
                    parts += [_lo(w), _hi(w)]
                tiles.append(jnp.concatenate(parts, axis=0))
            return tiles

        def body(g, x0):
            u = _layernorm(x0)
            store_group(wp, c, g, x0 + u * dsk)
            return u
        return chained(chains, get, body).astype(bf16)

    def m_tiles(c, ub, tiles, first=False, toks=None, at=None):
        for n in tiles:
            b_tile(c, ub, state, n, first, toks if n == at else None)
            tick(640)


    doA = "A" in MODE
    ub = {}

    def prep(c, chains=None):
        if doA:
            ub[c] = m1_prep(c, chains or CH_M1)

    def mm(c, tiles=range(NT), first=False):
        if doA:
            m_tiles(c, ub[c], tiles, first)

    def fk_(n):
        if doA:
            front_k(n)

    def fx_(n):
        if doA:
            front_x(n)

    wait(("x", 0), ("b", 0))
    start(("cv", 0))
    prep(0, CH_HEAD)
    mm(0, range(0, 2), True)
    wait(("b", 1))
    start(("x", 1))
    prep(1)
    mm(0, range(2, NT), True)
    prep(2)
    mm(1)
    wait(("cv", 0), ("x", 1))
    start(("cv", 1), ("x", 2), ("cv", 2))
    fk_(0); prep(3); mm(2); fx_(0)
    wait(("cv", 1), ("x", 2))
    start(("x", 3))
    fk_(1); prep(4); mm(3); fx_(1)
    wait(("cv", 2))
    start(("cv", 3), "c")
    fk_(2); prep(5); mm(4); fx_(2)
    wait(("cv", 3), ("x", 3))
    start(("cv", 4), *[("bar", i) for i in range(NBAR)])
    fk_(3); prep(6); mm(5); prep(7); mm(6); fx_(3)
    wait(("cv", 4))
    fk_(4)
    if X4LAST:
        mm(7); fx_(4)
    else:
        fx_(4); held = pending[-NB:]; del pending[-NB:]; mm(7); pending.extend(held)
    wait("c")
    if doA:
        pass
    elif "B" in MODE:
        for n in range(NT):
            for i in range(NB):
                pending.append((n, i))
        for _ in range(_p("SKIP", 44)):
            pending.pop(0)

    stretch[0] = STRETCH_B
    if "B" in MODE:
        carry = segment_carry(state)
        for c in range(NCH):
            y = _nt(fixup(c * CH, CH, carry, FIXSER_B), c_weights())
            for n in range(NT):
                wp[n, pl.ds(c * R, R), :] = wp[n, pl.ds(c * R, R), :] + _tile(y, n)
            tick(3200)
        drain()
    if not MERGE_BC:
        barrier()

    state[:] = [(zero, zero) for _ in range(NT)]
    if "C" in MODE and SPLIT_C:
        def stage_g(c, chains):
            def body(g, x1):
                x2 = x1 + _layernorm(x1) * gate_group(c, g)
                store_group(wp, c, g, x2)
                return x2
            chained(chains, lambda g: row_group(wp, c, g), body)

        def stage_u(c, chains):
            def body(g, x2):
                u = _layernorm(x2)
                store_group(wp, c, g, x2 + u * dsk)
                return u
            return chained(chains, lambda g: row_group(wp, c, g), body).astype(bf16)

        stage_g(0, CH_HEAD)
        nxt = stage_u(0, CH_HEAD)
        stage_g(1, CH_HEAD)
        for c in range(NCH):
            cur = nxt
            toks = None
            if c + 2 < NCH:
                stage_g(c + 2, CH_G)
                toks = list(last_toks)
            if c + 1 < NCH:
                nxt = stage_u(c + 1, CH_U)
            m_tiles(c, cur, range(NT), toks=toks, at=ANCH_G)
    elif "C" in MODE:
        for c in range(NCH):
            def body(g, x1):
                x2 = x1 + _layernorm(x1) * gate_group(c, g)
                u = _layernorm(x2)
                store_group(wp, c, g, x2 + u * dsk)
                return u
            ub2 = chained(CH_C0 if c == 0 else CH_M2, lambda g: row_group(wp, c, g), body).astype(bf16)
            m_tiles(c, ub2, range(NT))
    barrier()

    outs = []
    if "D" in MODE:
        carry = segment_carry(state)
        anchors = {}
        j0 = 0
        for c, nj in enumerate(D_STEPS):
            for k, t in enumerate(anchors.pop(c - ANCH_D, [])):
                carry[k % NT] = (carry[k % NT][0] + t, carry[k % NT][1])
            y = _nt(fixup(j0, nj, carry, FIXSER_D), c_weights())

            def get(g):
                return [t + y[g * GROWS:(g + 1) * GROWS, n * LN:(n + 1) * LN]
                        for n, t in enumerate(row_group(wp, 0, g, 8 * j0))]

            def body(g, x3):
                x4 = x3 + _layernorm(x3) * gate_group(0, g, j0)
                for n in range(NT):
                    for j in range(GROWS // 8):
                        ob[n, pl.ds(j0 + g * GROWS // 8 + j, SEG, stride=PF), :] = (
                            x4[8 * j:8 * j + 8, n * LN:(n + 1) * LN])
                return x4
            chained(CH_E2 if c + ANCH_D < len(D_STEPS) else CH_HEAD, get, body, 8 * nj, bool(FULL_D))
            anchors[c] = list(last_toks)
            for n in range(NT):
                for s in range(SEG):
                    cpy = pltpu.make_async_copy(
                        ob.at[n, pl.ds(s * PF + j0, nj), :],
                        out_hbm.at[0, pl.ds(s * J + j0, nj), pl.ds(n * LN, LN)], osem)
                    cpy.start()
                    outs.append(cpy)
            j0 += nj
        assert j0 == J
    while bar_idx[0] < NBAR:
        barrier()
    if MODE != "ABCD":
        for buf in (wp, hr, hi):
            pltpu.make_async_copy(buf.at[0], out_hbm.at[0, :, pl.ds(0, LN)], osem).start()
            pltpu.make_async_copy(buf.at[0], out_hbm.at[0, :, pl.ds(0, LN)], osem).wait()
        for buf in (gn,):
            pltpu.make_async_copy(buf.at[0, pl.ds(0, S)], out_hbm.at[0, :, pl.ds(0, LN)], osem).start()
            pltpu.make_async_copy(buf.at[0, pl.ds(0, S)], out_hbm.at[0, :, pl.ds(0, LN)], osem).wait()
        for buf in (xs, gs):
            pltpu.make_async_copy(buf.at[0], out_hbm.at[0, pl.ds(0, 256), pl.ds(0, LN)], osem).start()
            pltpu.make_async_copy(buf.at[0], out_hbm.at[0, pl.ds(0, 256), pl.ds(0, LN)], osem).wait()
    assert len(sem_of) <= 14 + NBAR
    assert not plans and not started, (plans.keys(), started.keys())
    if outs:
        pltpu.make_async_copy(out_hbm, out_hbm, osem).wait()


@jax.jit
def pallas_interleave_layers__ssm_conv_s5__ssm_conv_h3__prompt_kernel(
    A_x: jax.Array,
    A_Lambda_re: jax.Array,
    A_Lambda_im: jax.Array,
    A_B_re: jax.Array,
    A_B_im: jax.Array,
    A_C_re: jax.Array,
    A_C_im: jax.Array,
    A_log_dt: jax.Array,
    A_Dskip: jax.Array,
    B_q: jax.Array,
    B_k: jax.Array,
    B_v: jax.Array,
    B_shift_k: jax.Array,
    B_ssm_k: jax.Array,
    B_ssm_D: jax.Array,
):
    del B_q
    bf, f32, u32 = jnp.bfloat16, jnp.float32, jnp.uint32
    n_sems = 14 + NBAR
    hbm = pl.BlockSpec(memory_space=pl.ANY)
    return pl.pallas_call(
        _kernel,
        out_shape=jax.ShapeDtypeStruct((1, S, D), f32),
        in_specs=[hbm] * 17,
        out_specs=hbm,
        scratch_shapes=[
            pltpu.VMEM((D,), bf), pltpu.VMEM((D,), bf), pltpu.VMEM((D,), bf), pltpu.VMEM((D,), bf),
            pltpu.VMEM((4, D), bf), pltpu.VMEM((D,), bf),
            pltpu.VMEM((T, T), u32), pltpu.VMEM((T, T), u32), pltpu.VMEM((T // 2 + 8, 2 * T), u32),
            *[pltpu.VMEM((NT, SEG * (r1 - r0), LN), bf) for r0, r1 in X_PARTS],
            pltpu.VMEM((2, D, D), bf),
            pltpu.VMEM((2, D // 2, D), u32),
            pltpu.VMEM((2, NT, D, LN), bf),
            pltpu.VMEM((NT, KPAD + S, LN), bf),
            pltpu.VMEM((NT, S, LN), bf),
            pltpu.VMEM((NT, LN, S), bf),
            pltpu.VMEM((NB * NT, 2 * T, LN), f32),
            pltpu.VMEM((NB * NT, 2 * T, LN), f32),
            pltpu.VMEM((NB * NT, 2 * T, LN), f32),
            pltpu.VMEM((NT, SEG * PF, LN), f32),
            pltpu.VMEM((NT, S, LN), f32),
            pltpu.VMEM((NT, S, LN), f32),
            pltpu.VMEM((NT, S, LN), f32),
            pltpu.VMEM((NT, SEG * PF, LN), f32),
            pltpu.VMEM((NBAR, 16, LN), bf),
            pltpu.SemaphoreType.DMA((n_sems,)),
            pltpu.SemaphoreType.DMA(()),
        ],
        compiler_params=pltpu.CompilerParams(vmem_limit_bytes=112 * 1024 * 1024, flags={"XLA_TPU_EVENLY_DISTRIBUTE_CRITICAL_NODES": True}),
    )(A_Lambda_re, A_Lambda_im, A_log_dt, A_Dskip, B_shift_k.T, B_ssm_D, _FK, _FX, _INV,
      A_x, A_B_re, A_B_im, A_C_re, A_C_im, B_k, B_v, B_ssm_k)
```

```python
import numpy as np

import jax
import jax.numpy as jnp
from jax import lax
import jax.experimental.pallas as pl
import jax.experimental.pallas.tpu as pltpu

def _p(name, default):
    del name
    return default

MODE = _p("MODE", "ABCD")
S = 2048
D = 640
LN = 128
NT = D // LN
SEG = 8
J = S // SEG
CH = _p("CH", 32)
NCH = J // CH
R = SEG * CH
PW = J // 2 + 4
PF = J + 4
T = 128
NB = S // T
NQ = T // 8
EPS = 1e-5
X_PARTS = ((0, 104), (104, 144), (144, 216), (216, 256))
KPAD = 16
STRETCH_A = _p("SA", 6.2)
STRETCH_B = _p("SB", 3.4)
GROWS = _p("GROWS", 16)
CH_M1 = _p("CH_M1", 2)
CH_M2 = _p("CH_M2", 4)
CH_E2 = _p("CH_E2", 3)
FIXSER_B = _p("FIXSER_B", 0)
FIXSER_D = _p("FIXSER_D", 0)
NBAR = 6
ASTEP = _p("ASTEP", 32)
CSTEP = _p("CSTEP", 16)
BSTEP = _p("BSTEP", 32)
EARLY_B0 = _p("EARLY_B0", 1)
EARLY_C0 = _p("EARLY_C0", 1)
EVEN = _p("EVEN", 1)
MERGE_BC = _p("MERGE_BC", 0)
CH_C0 = _p("CH_C0", 8)
X4LAST = _p("X4LAST", 1)
MAC_CH = _p("MAC_CH", 1)
MAC_LONG = _p("MAC_LONG", 100)
FULL_D = _p("FULL_D", 1)
D_STEPS = [int(t) for t in _p("DSTEPS", "16,16,16,16,16,16,16,16,16,16,16,16,16,16,16,8,8").split(",")]
LAST_SPLIT = _p("LAST_SPLIT", 3)
ANCH_G = _p("ANCH_G", 3)
SPLIT_C = _p("SPLIT_C", 0)
CH_G = _p("CH_G", 4)
CH_U = _p("CH_U", 4)
ANCH_D = _p("ANCH_D", 3)
KTICK = _p("KTICK", 1.0)
XTICK = _p("XTICK", 0.0)
CH_HEAD = _p("CH_HEAD", 16)


def _pack_rows(a):
    u = np.asarray(a.astype(jnp.bfloat16)).view(np.uint16).astype(np.uint32)
    return u[0::2] | (u[1::2] << 16)


def _dft_constants():
    rho = np.arange(T)
    f = np.concatenate([np.arange(0, T, 2), np.arange(1, T, 2)])
    n = np.arange(T)
    theta = np.pi * np.outer(2 * f + 1, n) / (2 * T)
    c, s = np.cos(theta), -np.sin(theta)
    row_re = 16 * (rho // 8) + rho % 8
    row_im = row_re + 8
    fk = np.zeros((2 * T, T))
    fk[row_re] = c
    fk[row_im] = s
    kappa = np.arange(T)
    g, r = kappa // 16, kappa % 16
    t_of_kappa = np.where(r < 8, 16 * g + 2 * r, 16 * g + 2 * (r - 8) + 1)
    fx = fk[:, t_of_kappa]
    inv = np.zeros((T, 2 * T))
    inv[:, row_re] = c.T / T
    inv[:, row_im] = s.T / T
    inv = np.concatenate([inv, np.zeros((16, 2 * T))], axis=0)
    return _pack_rows(fk), _pack_rows(fx), _pack_rows(inv)


_FK, _FX, _INV = _dft_constants()

_NT_DIMS = (((1,), (1,)), ((), ()))


def _nt(a, b):
    return lax.dot_general(a, b, _NT_DIMS, preferred_element_type=jnp.float32)


def _nn(a, b):
    return jnp.dot(a, b, preferred_element_type=jnp.float32)


def _lo(w):
    return pltpu.bitcast(w << 16, jnp.float32)


def _hi(w):
    return pltpu.bitcast(w & jnp.uint32(0xFFFF0000), jnp.float32)


def _as_bf16(w):
    return pltpu.bitcast(w, jnp.bfloat16)


def _cmul(ar, ai, br, bi):
    return ar * br - ai * bi, ar * bi + ai * br


def _layernorm(x):
    m = jnp.mean(x, axis=-1, keepdims=True)
    d = x - m
    v = jnp.mean(d * d, axis=-1, keepdims=True)
    return d * lax.rsqrt(v + EPS)


def _tile(v, n):
    return v[:, n * LN:(n + 1) * LN]


def _kernel(lre_hbm, lim_hbm, ldt_hbm, dsk_hbm, sh_hbm, sd_hbm, fk_hbm, fx_hbm, inv_hbm,
            x_hbm, bre_hbm, bim_hbm, cre_hbm, cim_hbm, k_hbm, v_hbm, sk_hbm,
            out_hbm,
            lre_ref, lim_ref, ldt_ref, dsk_ref, sh_ref, sd_ref, fk_ref, fx_ref, inv_ref,
            xb0, xb1, xb2, xb3, braw, bw, cb, kb, vb, skb, xs, gs, ys, gn, wp, hr, hi, ob, bar,
            sems, osem):
    f32 = jnp.float32
    bf16 = jnp.bfloat16
    xbs = (xb0, xb1, xb2, xb3)
    xws = [b.bitcast(jnp.uint32) for b in xbs]
    cw = cb.bitcast(jnp.uint32)
    kw = kb.bitcast(jnp.uint32)
    vw = vb.bitcast(jnp.uint32)

    plans, started = {}, {}

    sem_of = {}

    def plan(group, src, dst):
        sem = sem_of.setdefault(group, len(sem_of))
        plans.setdefault(group, []).append(pltpu.make_async_copy(src, dst, sems.at[sem]))

    def start(*groups):
        for g in groups:
            started[g] = plans.pop(g)
            for c in started[g]:
                c.start()

    def wait(*groups):
        for g in groups:
            copies = started.pop(g)
            if g in fills:
                pltpu.make_async_copy(fills[g], fills[g], sems.at[sem_of[g]]).wait()
            else:
                for c in copies:
                    c.wait()

    for src, dst in ((lre_hbm, lre_ref), (lim_hbm, lim_ref), (ldt_hbm, ldt_ref), (dsk_hbm, dsk_ref),
                     (inv_hbm, inv_ref)):
        plan("par", src, dst)
    for src, dst in ((sh_hbm, sh_ref), (sd_hbm, sd_ref), (fk_hbm, fk_ref), (fx_hbm, fx_ref)):
        plan(("cv", 0), src, dst)
    fills = {}
    for p, (r0, r1) in enumerate(X_PARTS):
        fills["x", p] = xbs[p]
        for n in range(NT):
            for s in range(SEG):
                plan(("x", p), x_hbm.at[0, pl.ds(s * J + r0, r1 - r0), pl.ds(n * LN, LN)],
                     xbs[p].at[n, pl.ds(s * (r1 - r0), r1 - r0), :])
    fills["c"] = cb
    for n in range(NT):
        for i, src in enumerate((bre_hbm, bim_hbm)):
            plan(("b", 0 if n < 2 else 1), src.at[pl.ds(n * LN, LN), :], braw.at[i, pl.ds(n * LN, LN), :])
        col = pl.ds(n * LN, LN)
        plan(("cv", n), sk_hbm.at[col, :], skb.at[n])
        plan(("cv", n), k_hbm.at[0, :, col], kb.at[n, pl.ds(KPAD, S), :])
        plan(("cv", n), v_hbm.at[0, :, col], vb.at[n])
        for i, src in enumerate((cre_hbm, cim_hbm)):
            plan("c", src.at[:, col], cb.at[i, n])
    for i in range(NBAR):
        plan(("bar", i), bre_hbm.at[pl.ds(0, 16), pl.ds(0, LN)], bar.at[i])
    bar_idx = [0]

    def barrier():
        wait(("bar", bar_idx[0]))
        bar_idx[0] += 1

    start("par", ("x", 0), ("b", 0), ("b", 1))
    for n in range(NT):
        kb[n, 0:KPAD, :] = jnp.zeros((KPAD, LN), bf16)
    wait("par")

    def vec(ref):
        return ref[...].astype(f32).reshape(1, D)

    zmask = inv_ref[T // 2:T // 2 + 8, 0:LN]

    def token_of(v):
        return pltpu.bitcast(pltpu.bitcast(v, jnp.uint32) & zmask, f32)

    def token_of_all(v):
        z = zmask
        for r in range(v.shape[0] // 8):
            for n in range(v.shape[1] // LN):
                z = z & pltpu.bitcast(v[8 * r:8 * r + 8, n * LN:(n + 1) * LN], jnp.uint32)
        return pltpu.bitcast(z, f32)

    lre, lim = vec(lre_ref), vec(lim_ref)
    dt = jnp.exp(vec(ldt_ref)).astype(bf16).astype(f32)
    ar, ai = dt * lre, dt * lim
    mag = jnp.exp(ar)
    lr1, li1 = mag * jnp.cos(ai), mag * jnp.sin(ai)
    den = lre * lre + lim * lim
    nr = lr1 - 1.0
    s2r = 2.0 * ((nr * lre + li1 * lim) / den)
    s2i = 2.0 * ((li1 * lre - nr * lim) / den)
    lr = jnp.broadcast_to(lr1, (SEG, D))
    li = jnp.broadcast_to(-li1, (SEG, D))
    s_cols = [tuple(jnp.broadcast_to(_tile(v, n), (LN, LN)).T for v in (s2r, s2i)) for n in range(NT)]
    dsk = vec(dsk_ref)
    sub = lax.broadcasted_iota(jnp.int32, (SEG, LN), 0)

    def shifted(v, k):
        return jnp.where(sub >= k, pltpu.roll(v, k, 0), 0.0)

    def segment_carry(state):
        pr, pi = lr, li
        for _ in range(J.bit_length() - 1):
            pr, pi = pr * pr - pi * pi, 2.0 * pr * pi
        pws = [(pr, pi)]
        for _ in range(2):
            pr, pi = pr * pr - pi * pi, 2.0 * pr * pi
            pws.append((pr, pi))
        out = []
        for n, (er, ei) in enumerate(state):
            cr, ci = shifted(er, 1), shifted(ei, 1)
            for k, (ar_, ai_) in zip((1, 2, 4), pws):
                tr, ti = _cmul(_tile(ar_, n), _tile(ai_, n), shifted(cr, k), shifted(ci, k))
                cr, ci = cr + tr, ci + ti
            out.append((cr, ci))
        return out

    last_toks = []

    def chained(chains, get_group, body, rows=R, full=False):
        toks = [None] * chains
        res = []
        for g in range(rows // GROWS):
            tiles = get_group(g)
            t = toks[g % chains]
            if t is not None:
                tiles[0] = tiles[0] + jnp.concatenate([t] * (GROWS // 8), axis=0)
            out = body(g, jnp.concatenate(tiles, axis=1))
            toks[g % chains] = token_of_all(out) if full else token_of(out[0:8, 0:LN])
            res.append(out)
        last_toks[:] = [t for t in toks if t is not None]
        return jnp.concatenate(res, axis=0)

    def anchored(words, toks):
        if not toks:
            return words
        z = pltpu.bitcast(toks[0], jnp.uint32)
        for t in toks[1:]:
            z = z | pltpu.bitcast(t, jnp.uint32)
        top = jnp.concatenate([words[0:8, 0:LN] | z, words[0:8, LN:]], axis=1)
        return jnp.concatenate([top, words[8:]], axis=0)

    def b_tile(j0, nj, ub, state, n, first=False, toks=None):
        if first:
            a, b = s_cols[n]
            parts = ([], [])
            for r in range(LN // 32):
                rows = pl.ds(n * LN + 32 * r, 32)
                b_re, b_im = braw[0, rows, :].astype(f32), braw[1, rows, :].astype(f32)
                ar_ = jnp.concatenate([a[32 * r:32 * r + 32]] * NT, axis=1)
                bi_ = jnp.concatenate([b[32 * r:32 * r + 32]] * NT, axis=1)
                for i, val in enumerate((b_re * ar_ - b_im * bi_, -(b_re * bi_ + b_im * ar_))):
                    packed = val.astype(bf16)
                    bw[i, pl.ds(n * (LN // 2) + 16 * r, 16), :] = pltpu.bitcast(packed, jnp.uint32)
                    parts[i].append(packed)
            halves = [jnp.concatenate(p, axis=0) for p in parts]
        else:
            halves = [_as_bf16(anchored(bw[i, pl.ds(n * (LN // 2), LN // 2), :], toks if i == 0 else None))
                      for i in range(2)]
        bu = _nt(ub, jnp.concatenate(halves, axis=0))
        sr, si = state[n]
        l_r, l_i = _tile(lr, n), _tile(li, n)
        for j in range(nj):
            mr, mi = _cmul(l_r, l_i, sr, si)
            sr = mr + bu[8 * j:8 * j + 8, :LN]
            si = mi + bu[8 * j:8 * j + 8, LN:]
            hr[n, pl.ds(8 * (j0 + j), 8), :] = sr
            hi[n, pl.ds(8 * (j0 + j), 8), :] = si
        state[n] = (sr, si)

    def fixup(j0, nj, carry, FIXSER=0):
        cols = []
        tok = None
        for n in range(NT):
            cr, ci = carry[n]
            if tok is not None and FIXSER:
                cr = cr + tok
                ci = ci + tok
            l_r, l_i = _tile(lr, n), _tile(li, n)
            pr, pi = [], []
            for j in range(j0, j0 + nj):
                cr, ci = _cmul(l_r, l_i, cr, ci)
                pr.append(hr[n, pl.ds(8 * j, 8), :] + cr)
                pi.append(hi[n, pl.ds(8 * j, 8), :] + ci)
            carry[n] = (cr, ci)
            if FIXSER:
                tok = token_of(cr)
            cols.append(jnp.concatenate(pr, axis=0))
            cols.append(jnp.concatenate(pi, axis=0))
        return jnp.concatenate(cols, axis=1).astype(bf16)

    def c_weights():
        return jnp.concatenate([_as_bf16(cw[k % 2, k // 2]) for k in range(2 * NT)], axis=1)

    def row_group(ref, j0, g):
        return [ref[n, pl.ds(8 * j0 + g * GROWS, GROWS), :] for n in range(NT)]

    def gate_group(j0, g):
        j0 = j0 + g * GROWS // 8
        return jnp.concatenate(
            [jnp.concatenate([gn[n, pl.ds(j0 + j, SEG, stride=PF), :] for j in range(GROWS // 8)],
                             axis=0) for n in range(NT)], axis=1)

    def store_group(ref, j0, g, val):
        for n in range(NT):
            ref[n, pl.ds(8 * j0 + g * GROWS, GROWS), :] = _tile(val, n)

    token = [None] * MAC_CH

    def mac_site(n, i, q):
        re_rows, im_rows = pl.ds(16 * q, 8), pl.ds(16 * q + 8, 8)
        yr = yi = token[q % MAC_CH]
        for m in range(i + 1):
            gr, gi = gs[m * NT + n, re_rows, :], gs[m * NT + n, im_rows, :]
            xr, xi = xs[(i - m) * NT + n, re_rows, :], xs[(i - m) * NT + n, im_rows, :]
            if yr is None:
                yr, yi = _cmul(gr, gi, xr, xi)
            elif m % MAC_LONG == 0:
                yr = (yr + gr * xr) - gi * xi
                yi = (yi + gr * xi) + gi * xr
            else:
                tr, ti = _cmul(gr, gi, xr, xi)
                yr, yi = yr + tr, yi + ti
        ys[i * NT + n, re_rows, :] = yr
        ys[i * NT + n, im_rows, :] = yi
        token[q % MAC_CH] = token_of(yr + yi)

    def conv_block(n, i):
        for q in range(NQ):
            mac_site(n, i, q)
        z = ys[i * NT + n]
        if i > 0:
            zp = ys[(i - 1) * NT + n]
            parts = []
            for q in range(NQ):
                re, im = z[16 * q:16 * q + 8], z[16 * q + 8:16 * q + 16]
                pre, pim = zp[16 * q:16 * q + 8], zp[16 * q + 8:16 * q + 16]
                parts += [re - pim, im + pre] if q < NQ // 2 else [re + pim, im - pre]
            z = jnp.concatenate(parts, axis=0)
        y = _nn(_as_bf16(inv_ref[0:T // 2, :]), z.astype(bf16))
        gn[n, pl.ds((i * T // J) * PF + (i * T) % J, T), :] = y

    pending = []
    credit = [0.0]
    stretch = [STRETCH_A]

    def tick(cycles):
        if not pending:
            credit[0] = 0.0
            return
        credit[0] += cycles
        while pending and credit[0] >= stretch[0] * NQ * (pending[0][1] + 1):
            n, i = pending.pop(0)
            credit[0] -= stretch[0] * NQ * (i + 1) - 64
            conv_block(n, i)

    def drain():
        while pending:
            conv_block(*pending.pop(0))

    def front_k(n):
        sd = jnp.broadcast_to(_tile(vec(sd_ref), n), (8, LN))
        fk = _as_bf16(fk_ref[...])
        for m in range(NB):
            kf = _nt(fk, skb[n, :, pl.ds(m * T, T)])
            if m == 0:
                kf = jnp.concatenate(
                    [kf[8 * r:8 * r + 8] + sd if r % 2 == 0 else kf[8 * r:8 * r + 8]
                     for r in range(2 * NQ)], axis=0)
            gs[m * NT + n] = kf
            tick(64 * KTICK)

    def front_x(n):
        taps = sh_ref[...].astype(f32)
        fx = _as_bf16(fx_ref[...])
        a0, a1, a2, a3 = (jnp.broadcast_to(_tile(taps[i:i + 1], n), (T // 2, LN)) for i in range(4))
        for m in range(NB):
            base = KPAD // 2 + m * (T // 2)
            w0 = kw[n, pl.ds(base, T // 2), :]
            w1 = kw[n, pl.ds(base - 1, T // 2), :]
            w2 = kw[n, pl.ds(base - 2, T // 2), :]
            k0, k1, k2, k3, k4 = _hi(w0), _lo(w0), _hi(w1), _lo(w1), _hi(w2)
            vv = vw[n, pl.ds(m * (T // 2), T // 2), :]
            even = (a3 * k4 + a2 * k3 + a1 * k2 + a0 * k1) * _lo(vv)
            odd = (a3 * k3 + a2 * k2 + a1 * k1 + a0 * k0) * _hi(vv)
            parts = []
            for g in range(T // 16):
                parts += [even[8 * g:8 * g + 8], odd[8 * g:8 * g + 8]]
            xs[m * NT + n] = _nn(fx, jnp.concatenate(parts, axis=0).astype(bf16))
            tick(64 * XTICK)
        for i in range(NB):
            pending.append((n, i))

    zero = jnp.zeros((SEG, LN), f32)
    state = [(zero, zero) for _ in range(NT)]

    def m1_prep(j0, nj, chains):
        def get(g):
            tiles = []
            for n in range(NT):
                parts = []
                for q in range(GROWS // 16):
                    row = j0 + g * GROWS // 8 + 2 * q
                    p = max(i for i, (r0, _) in enumerate(X_PARTS) if r0 <= row)
                    r0, r1 = X_PARTS[p]
                    w = xws[p][n, pl.ds((row - r0) // 2, SEG, stride=(r1 - r0) // 2), :]
                    parts += [_lo(w), _hi(w)]
                tiles.append(jnp.concatenate(parts, axis=0))
            return tiles

        def body(g, x0):
            u = _layernorm(x0)
            store_group(wp, j0, g, x0 + u * dsk)
            return u
        return chained(chains, get, body, 8 * nj).astype(bf16)

    def m_tiles(j0, nj, ub, tiles, first=False):
        for n in tiles:
            b_tile(j0, nj, ub, state, n, first)
            tick(20 * nj)


    doA = "A" in MODE
    ub = {}

    def pieces(c):
        return [(c * CH + k * ASTEP, ASTEP) for k in range(CH // ASTEP)]

    def prep(c, chains=None):
        if doA:
            for j0, nj in pieces(c):
                ub[j0] = m1_prep(j0, nj, chains or CH_M1)

    def mm(c, tiles=range(NT), first=False):
        if doA:
            for k, (j0, nj) in enumerate(pieces(c)):
                m_tiles(j0, nj, ub[j0], tiles, first and k == 0)

    def fk_(n):
        if doA:
            front_k(n)

    def fx_(n):
        if doA:
            front_x(n)

    wait(("x", 0), ("b", 0))
    start(("cv", 0))
    prep(0, CH_HEAD)
    mm(0, range(0, 2), True)
    wait(("b", 1))
    start(("x", 1))
    prep(1)
    mm(0, range(2, NT), True)
    prep(2)
    mm(1)
    wait(("cv", 0), ("x", 1))
    start(("cv", 1), ("x", 2), ("cv", 2))
    fk_(0); prep(3); mm(2); fx_(0)
    wait(("cv", 1), ("x", 2))
    start(("x", 3))
    fk_(1); prep(4); mm(3); fx_(1)
    wait(("cv", 2))
    start(("cv", 3), "c")
    fk_(2); prep(5); mm(4); fx_(2)
    wait(("cv", 3), ("x", 3))
    start(("cv", 4), *[("bar", i) for i in range(NBAR)])
    fk_(3); prep(6); mm(5); prep(7); mm(6); fx_(3)
    wait(("cv", 4))
    fk_(4)
    if X4LAST:
        mm(7); fx_(4)
    else:
        fx_(4); held = pending[-NB:]; del pending[-NB:]; mm(7); pending.extend(held)
    if "B" in MODE and EARLY_B0:
        carry = segment_carry(state)
        h0 = fixup(0, BSTEP, carry, FIXSER_B)
    wait("c")
    if doA:
        pass
    elif "B" in MODE:
        for n in range(NT):
            for i in range(NB):
                pending.append((n, i))
        for _ in range(_p("SKIP", 44)):
            pending.pop(0)

    stretch[0] = STRETCH_B
    credit[0] = min(credit[0], 1000.0)
    if "B" in MODE:
        if not EARLY_B0:
            carry = segment_carry(state)
        for j0 in range(0, J, BSTEP):
            h = h0 if j0 == 0 and EARLY_B0 else fixup(j0, BSTEP, carry, FIXSER_B)
            y = _nt(h, c_weights())
            rows = pl.ds(8 * j0, 8 * BSTEP)
            for n in range(NT):
                wp[n, rows, :] = wp[n, rows, :] + _tile(y, n)
            tick(100 * BSTEP)
        drain()
    def prep2(j0, chains):
        def body(g, x1):
            x2 = x1 + _layernorm(x1) * gate_group(j0, g)
            u = _layernorm(x2)
            store_group(wp, j0, g, x2 + u * dsk)
            return u
        return chained(chains, lambda g: row_group(wp, j0, g), body, 8 * CSTEP).astype(bf16)

    if "C" in MODE and EARLY_C0:
        ub2 = prep2(0, CH_C0)
    barrier()

    state[:] = [(zero, zero) for _ in range(NT)]
    if "C" in MODE:
        for j0 in range(0, J, CSTEP):
            if j0 > 0 or not EARLY_C0:
                ub2 = prep2(j0, CH_C0 if j0 == 0 else CH_M2)
            m_tiles(j0, CSTEP, ub2, range(NT))
    barrier()

    outs = []
    if "D" in MODE:
        carry = segment_carry(state)
        anchors = {}
        j0 = 0
        for c, nj in enumerate(D_STEPS):
            for k, t in enumerate(anchors.pop(c - ANCH_D, [])):
                carry[k % NT] = (carry[k % NT][0] + t, carry[k % NT][1])
            y = _nt(fixup(j0, nj, carry, FIXSER_D), c_weights())

            def get(g):
                return [t + y[g * GROWS:(g + 1) * GROWS, n * LN:(n + 1) * LN]
                        for n, t in enumerate(row_group(wp, j0, g))]

            def body(g, x3):
                x4 = x3 + _layernorm(x3) * gate_group(j0, g)
                for n in range(NT):
                    for j in range(GROWS // 8):
                        ob[n, pl.ds(j0 + g * GROWS // 8 + j, SEG, stride=PF), :] = (
                            x4[8 * j:8 * j + 8, n * LN:(n + 1) * LN])
                return x4
            chained(CH_E2 if c + ANCH_D < len(D_STEPS) else CH_HEAD, get, body, 8 * nj, bool(FULL_D))
            anchors[c] = list(last_toks)
            for n in range(NT):
                for s in range(SEG):
                    cpy = pltpu.make_async_copy(
                        ob.at[n, pl.ds(s * PF + j0, nj), :],
                        out_hbm.at[0, pl.ds(s * J + j0, nj), pl.ds(n * LN, LN)], osem)
                    cpy.start()
                    outs.append(cpy)
            j0 += nj
        assert j0 == J
    while bar_idx[0] < NBAR:
        barrier()
    if MODE != "ABCD":
        for buf in (wp, hr, hi):
            pltpu.make_async_copy(buf.at[0], out_hbm.at[0, :, pl.ds(0, LN)], osem).start()
            pltpu.make_async_copy(buf.at[0], out_hbm.at[0, :, pl.ds(0, LN)], osem).wait()
        for buf in (gn,):
            pltpu.make_async_copy(buf.at[0, pl.ds(0, S)], out_hbm.at[0, :, pl.ds(0, LN)], osem).start()
            pltpu.make_async_copy(buf.at[0, pl.ds(0, S)], out_hbm.at[0, :, pl.ds(0, LN)], osem).wait()
        for buf in (xs, gs):
            pltpu.make_async_copy(buf.at[0], out_hbm.at[0, pl.ds(0, 256), pl.ds(0, LN)], osem).start()
            pltpu.make_async_copy(buf.at[0], out_hbm.at[0, pl.ds(0, 256), pl.ds(0, LN)], osem).wait()
    assert len(sem_of) <= 14 + NBAR
    assert not plans and not started, (plans.keys(), started.keys())
    if outs:
        pltpu.make_async_copy(out_hbm, out_hbm, osem).wait()


@jax.jit
def pallas_interleave_layers__ssm_conv_s5__ssm_conv_h3__prompt_kernel(
    A_x: jax.Array,
    A_Lambda_re: jax.Array,
    A_Lambda_im: jax.Array,
    A_B_re: jax.Array,
    A_B_im: jax.Array,
    A_C_re: jax.Array,
    A_C_im: jax.Array,
    A_log_dt: jax.Array,
    A_Dskip: jax.Array,
    B_q: jax.Array,
    B_k: jax.Array,
    B_v: jax.Array,
    B_shift_k: jax.Array,
    B_ssm_k: jax.Array,
    B_ssm_D: jax.Array,
):
    del B_q
    bf, f32, u32 = jnp.bfloat16, jnp.float32, jnp.uint32
    n_sems = 14 + NBAR
    hbm = pl.BlockSpec(memory_space=pl.ANY)
    return pl.pallas_call(
        _kernel,
        out_shape=jax.ShapeDtypeStruct((1, S, D), f32),
        in_specs=[hbm] * 17,
        out_specs=hbm,
        scratch_shapes=[
            pltpu.VMEM((D,), bf), pltpu.VMEM((D,), bf), pltpu.VMEM((D,), bf), pltpu.VMEM((D,), bf),
            pltpu.VMEM((4, D), bf), pltpu.VMEM((D,), bf),
            pltpu.VMEM((T, T), u32), pltpu.VMEM((T, T), u32), pltpu.VMEM((T // 2 + 8, 2 * T), u32),
            *[pltpu.VMEM((NT, SEG * (r1 - r0), LN), bf) for r0, r1 in X_PARTS],
            pltpu.VMEM((2, D, D), bf),
            pltpu.VMEM((2, D // 2, D), u32),
            pltpu.VMEM((2, NT, D, LN), bf),
            pltpu.VMEM((NT, KPAD + S, LN), bf),
            pltpu.VMEM((NT, S, LN), bf),
            pltpu.VMEM((NT, LN, S), bf),
            pltpu.VMEM((NB * NT, 2 * T, LN), f32),
            pltpu.VMEM((NB * NT, 2 * T, LN), f32),
            pltpu.VMEM((NB * NT, 2 * T, LN), f32),
            pltpu.VMEM((NT, SEG * PF, LN), f32),
            pltpu.VMEM((NT, S, LN), f32),
            pltpu.VMEM((NT, S, LN), f32),
            pltpu.VMEM((NT, S, LN), f32),
            pltpu.VMEM((NT, SEG * PF, LN), f32),
            pltpu.VMEM((NBAR, 16, LN), bf),
            pltpu.SemaphoreType.DMA((n_sems,)),
            pltpu.SemaphoreType.DMA(()),
        ],
        compiler_params=pltpu.CompilerParams(
            vmem_limit_bytes=112 * 1024 * 1024,
            flags={"XLA_TPU_EVENLY_DISTRIBUTE_CRITICAL_NODES": True} if EVEN else {}),
    )(A_Lambda_re, A_Lambda_im, A_log_dt, A_Dskip, B_shift_k.T, B_ssm_D, _FK, _FX, _INV,
      A_x, A_B_re, A_B_im, A_C_re, A_C_im, B_k, B_v, B_ssm_k)
```

```python
import numpy as np

import jax
import jax.numpy as jnp
from jax import lax
import jax.experimental.pallas as pl
import jax.experimental.pallas.tpu as pltpu

S = 2048
D = 640
LN = 128
NT = D // LN
SEG = 8
J = S // SEG
PF = J + 4
T = 128
NB = S // T
NQ = T // 8
EPS = 1e-5
KPAD = 16
X_PARTS = ((0, 104), (104, 144), (144, 216), (216, 256))
GROWS = 16
A_STEP, A_CHAINS = 32, 2
B_STEP = 32
C_STEP, C_CHAINS, C0_CHAINS = 16, 4, 8
D_STEPS, D_CHAINS, D_LAG = (16,) * 15 + (8, 8), 3, 3
WIDE = 16
STRETCH_A, STRETCH_B = 6.2, 3.5
NBAR = 2


def _pack_rows(a):
    u = np.asarray(a.astype(jnp.bfloat16)).view(np.uint16).astype(np.uint32)
    return u[0::2] | (u[1::2] << 16)


def _dft_constants():
    rho = np.arange(T)
    f = np.concatenate([np.arange(0, T, 2), np.arange(1, T, 2)])
    n = np.arange(T)
    theta = np.pi * np.outer(2 * f + 1, n) / (2 * T)
    c, s = np.cos(theta), -np.sin(theta)
    row_re = 16 * (rho // 8) + rho % 8
    row_im = row_re + 8
    fk = np.zeros((2 * T, T))
    fk[row_re] = c
    fk[row_im] = s
    kappa = np.arange(T)
    g, r = kappa // 16, kappa % 16
    t_of_kappa = np.where(r < 8, 16 * g + 2 * r, 16 * g + 2 * (r - 8) + 1)
    fx = fk[:, t_of_kappa]
    inv = np.zeros((T, 2 * T))
    inv[:, row_re] = c.T / T
    inv[:, row_im] = s.T / T
    inv = np.concatenate([inv, np.zeros((16, 2 * T))], axis=0)
    return _pack_rows(fk), _pack_rows(fx), _pack_rows(inv)


_FK, _FX, _INV = _dft_constants()

_NT_DIMS = (((1,), (1,)), ((), ()))


def _nt(a, b):
    return lax.dot_general(a, b, _NT_DIMS, preferred_element_type=jnp.float32)


def _nn(a, b):
    return jnp.dot(a, b, preferred_element_type=jnp.float32)


def _lo(w):
    return pltpu.bitcast(w << 16, jnp.float32)


def _hi(w):
    return pltpu.bitcast(w & jnp.uint32(0xFFFF0000), jnp.float32)


def _as_bf16(w):
    return pltpu.bitcast(w, jnp.bfloat16)


def _cmul(ar, ai, br, bi):
    return ar * br - ai * bi, ar * bi + ai * br


def _layernorm(x):
    m = jnp.mean(x, axis=-1, keepdims=True)
    d = x - m
    v = jnp.mean(d * d, axis=-1, keepdims=True)
    return d * jnp.exp2(-0.5 * jnp.log2(v + EPS))


def _tile(v, n):
    return v[:, n * LN:(n + 1) * LN]


def _kernel(lre_hbm, lim_hbm, ldt_hbm, dsk_hbm, sh_hbm, sd_hbm, fk_hbm, fx_hbm, inv_hbm,
            x_hbm, bre_hbm, bim_hbm, cre_hbm, cim_hbm, k_hbm, v_hbm, sk_hbm,
            out_hbm,
            lre_ref, lim_ref, ldt_ref, dsk_ref, sh_ref, sd_ref, fk_ref, fx_ref, inv_ref,
            xb0, xb1, xb2, xb3, braw, bw, cb, kb, vb, skb, xs, gs, ys, gn, wp, hr, hi, ob, bar,
            sems, osem):
    f32 = jnp.float32
    bf16 = jnp.bfloat16
    xbs = (xb0, xb1, xb2, xb3)
    xws = [b.bitcast(jnp.uint32) for b in xbs]
    cw = cb.bitcast(jnp.uint32)
    kw = kb.bitcast(jnp.uint32)
    vw = vb.bitcast(jnp.uint32)

    plans, started, sem_of = {}, {}, {}

    def plan(group, src, dst):
        sem = sem_of.setdefault(group, len(sem_of))
        plans.setdefault(group, []).append(pltpu.make_async_copy(src, dst, sems.at[sem]))

    def start(*groups):
        for g in groups:
            started[g] = plans.pop(g)
            for c in started[g]:
                c.start()

    def wait(*groups):
        for g in groups:
            copies = started.pop(g)
            if g in fills:
                pltpu.make_async_copy(fills[g], fills[g], sems.at[sem_of[g]]).wait()
            else:
                for c in copies:
                    c.wait()

    for src, dst in ((lre_hbm, lre_ref), (lim_hbm, lim_ref), (ldt_hbm, ldt_ref), (dsk_hbm, dsk_ref),
                     (inv_hbm, inv_ref)):
        plan("par", src, dst)
    for src, dst in ((sh_hbm, sh_ref), (sd_hbm, sd_ref), (fk_hbm, fk_ref), (fx_hbm, fx_ref)):
        plan(("cv", 0), src, dst)
    fills = {}
    for p, (r0, r1) in enumerate(X_PARTS):
        fills["x", p] = xbs[p]
        for n in range(NT):
            for s in range(SEG):
                plan(("x", p), x_hbm.at[0, pl.ds(s * J + r0, r1 - r0), pl.ds(n * LN, LN)],
                     xbs[p].at[n, pl.ds(s * (r1 - r0), r1 - r0), :])
    fills["c"] = cb
    for n in range(NT):
        for i, src in enumerate((bre_hbm, bim_hbm)):
            plan(("b", 0 if n < 2 else 1), src.at[pl.ds(n * LN, LN), :], braw.at[i, pl.ds(n * LN, LN), :])
        col = pl.ds(n * LN, LN)
        plan(("cv", n), sk_hbm.at[col, :], skb.at[n])
        plan(("cv", n), k_hbm.at[0, :, col], kb.at[n, pl.ds(KPAD, S), :])
        plan(("cv", n), v_hbm.at[0, :, col], vb.at[n])
        for i, src in enumerate((cre_hbm, cim_hbm)):
            plan("c", src.at[:, col], cb.at[i, n])
    for i in range(NBAR):
        plan(("bar", i), bre_hbm.at[pl.ds(0, 16), pl.ds(0, LN)], bar.at[i])
    bar_idx = [0]

    def barrier():
        wait(("bar", bar_idx[0]))
        bar_idx[0] += 1

    start("par", ("x", 0), ("b", 0), ("b", 1))
    for n in range(NT):
        kb[n, 0:KPAD, :] = jnp.zeros((KPAD, LN), bf16)
    wait("par")

    def vec(ref):
        return ref[...].astype(f32).reshape(1, D)

    zmask = inv_ref[T // 2:T // 2 + 8, 0:LN]

    def token_of(v):
        return pltpu.bitcast(pltpu.bitcast(v, jnp.uint32) & zmask, f32)

    def token_of_all(v):
        z = zmask
        for r in range(v.shape[0] // 8):
            for n in range(v.shape[1] // LN):
                z = z & pltpu.bitcast(v[8 * r:8 * r + 8, n * LN:(n + 1) * LN], jnp.uint32)
        return pltpu.bitcast(z, f32)

    lre, lim = vec(lre_ref), vec(lim_ref)
    dt = jnp.exp(vec(ldt_ref)).astype(bf16).astype(f32)
    ar, ai = dt * lre, dt * lim
    mag = jnp.exp(ar)
    lr1, li1 = mag * jnp.cos(ai), mag * jnp.sin(ai)
    den = lre * lre + lim * lim
    nr = lr1 - 1.0
    s2r = 2.0 * ((nr * lre + li1 * lim) / den)
    s2i = 2.0 * ((li1 * lre - nr * lim) / den)
    lr = jnp.broadcast_to(lr1, (SEG, D))
    li = jnp.broadcast_to(-li1, (SEG, D))
    s_cols = [tuple(jnp.broadcast_to(_tile(v, n), (LN, LN)).T for v in (s2r, s2i)) for n in range(NT)]
    dsk = vec(dsk_ref)
    sub = lax.broadcasted_iota(jnp.int32, (SEG, LN), 0)

    def shifted(v, k):
        return jnp.where(sub >= k, pltpu.roll(v, k, 0), 0.0)

    def segment_carry(state):
        pr, pi = lr, li
        for _ in range(J.bit_length() - 1):
            pr, pi = pr * pr - pi * pi, 2.0 * pr * pi
        pws = [(pr, pi)]
        for _ in range(2):
            pr, pi = pr * pr - pi * pi, 2.0 * pr * pi
            pws.append((pr, pi))
        out = []
        for n, (er, ei) in enumerate(state):
            cr, ci = shifted(er, 1), shifted(ei, 1)
            for k, (ar_, ai_) in zip((1, 2, 4), pws):
                tr, ti = _cmul(_tile(ar_, n), _tile(ai_, n), shifted(cr, k), shifted(ci, k))
                cr, ci = cr + tr, ci + ti
            out.append((cr, ci))
        return out

    last_toks = []

    def chained(chains, get_group, body, rows, full=False):
        toks = [None] * chains
        res = []
        for g in range(rows // GROWS):
            tiles = get_group(g)
            t = toks[g % chains]
            if t is not None:
                tiles[0] = tiles[0] + jnp.concatenate([t] * (GROWS // 8), axis=0)
            out = body(g, jnp.concatenate(tiles, axis=1))
            toks[g % chains] = token_of_all(out) if full else token_of(out[0:8, 0:LN])
            res.append(out)
        last_toks[:] = [t for t in toks if t is not None]
        return jnp.concatenate(res, axis=0)

    def b_tile(j0, nj, ub, n, first=False):
        if first:
            a, b = s_cols[n]
            parts = ([], [])
            for r in range(LN // 32):
                rows = pl.ds(n * LN + 32 * r, 32)
                b_re, b_im = braw[0, rows, :].astype(f32), braw[1, rows, :].astype(f32)
                ar_ = jnp.concatenate([a[32 * r:32 * r + 32]] * NT, axis=1)
                bi_ = jnp.concatenate([b[32 * r:32 * r + 32]] * NT, axis=1)
                for i, val in enumerate((b_re * ar_ - b_im * bi_, -(b_re * bi_ + b_im * ar_))):
                    packed = val.astype(bf16)
                    bw[i, pl.ds(n * (LN // 2) + 16 * r, 16), :] = pltpu.bitcast(packed, jnp.uint32)
                    parts[i].append(packed)
            halves = [jnp.concatenate(p, axis=0) for p in parts]
        else:
            halves = [_as_bf16(bw[i, pl.ds(n * (LN // 2), LN // 2), :]) for i in range(2)]
        bu = _nt(ub, jnp.concatenate(halves, axis=0))
        sr, si = state[n]
        l_r, l_i = _tile(lr, n), _tile(li, n)
        for j in range(nj):
            mr, mi = _cmul(l_r, l_i, sr, si)
            sr = mr + bu[8 * j:8 * j + 8, :LN]
            si = mi + bu[8 * j:8 * j + 8, LN:]
            hr[n, pl.ds(8 * (j0 + j), 8), :] = sr
            hi[n, pl.ds(8 * (j0 + j), 8), :] = si
        state[n] = (sr, si)

    def fixup(j0, nj, carry):
        cols = []
        for n in range(NT):
            cr, ci = carry[n]
            l_r, l_i = _tile(lr, n), _tile(li, n)
            pr, pi = [], []
            for j in range(j0, j0 + nj):
                cr, ci = _cmul(l_r, l_i, cr, ci)
                pr.append(hr[n, pl.ds(8 * j, 8), :] + cr)
                pi.append(hi[n, pl.ds(8 * j, 8), :] + ci)
            carry[n] = (cr, ci)
            cols.append(jnp.concatenate(pr, axis=0))
            cols.append(jnp.concatenate(pi, axis=0))
        return jnp.concatenate(cols, axis=1).astype(bf16)

    def c_weights():
        return jnp.concatenate([_as_bf16(cw[k % 2, k // 2]) for k in range(2 * NT)], axis=1)

    def row_group(ref, j0, g):
        return [ref[n, pl.ds(8 * j0 + g * GROWS, GROWS), :] for n in range(NT)]

    def gate_group(j0, g):
        j0 = j0 + g * GROWS // 8
        return jnp.concatenate(
            [jnp.concatenate([gn[n, pl.ds(j0 + j, SEG, stride=PF), :] for j in range(GROWS // 8)],
                             axis=0) for n in range(NT)], axis=1)

    def store_group(ref, j0, g, val):
        for n in range(NT):
            ref[n, pl.ds(8 * j0 + g * GROWS, GROWS), :] = _tile(val, n)

    token = [None]

    def mac_site(n, i, q):
        re_rows, im_rows = pl.ds(16 * q, 8), pl.ds(16 * q + 8, 8)
        yr = yi = token[0]
        for m in range(i + 1):
            gr, gi = gs[m * NT + n, re_rows, :], gs[m * NT + n, im_rows, :]
            xr, xi = xs[(i - m) * NT + n, re_rows, :], xs[(i - m) * NT + n, im_rows, :]
            if yr is None:
                yr, yi = _cmul(gr, gi, xr, xi)
            elif m == 0:
                yr = (yr + gr * xr) - gi * xi
                yi = (yi + gr * xi) + gi * xr
            else:
                tr, ti = _cmul(gr, gi, xr, xi)
                yr, yi = yr + tr, yi + ti
        ys[i * NT + n, re_rows, :] = yr
        ys[i * NT + n, im_rows, :] = yi
        token[0] = token_of(yr + yi)

    def conv_block(n, i):
        for q in range(NQ):
            mac_site(n, i, q)
        z = ys[i * NT + n]
        if i > 0:
            zp = ys[(i - 1) * NT + n]
            parts = []
            for q in range(NQ):
                re, im = z[16 * q:16 * q + 8], z[16 * q + 8:16 * q + 16]
                pre, pim = zp[16 * q:16 * q + 8], zp[16 * q + 8:16 * q + 16]
                parts += [re - pim, im + pre] if q < NQ // 2 else [re + pim, im - pre]
            z = jnp.concatenate(parts, axis=0)
        y = _nn(_as_bf16(inv_ref[0:T // 2, :]), z.astype(bf16))
        gn[n, pl.ds((i * T // J) * PF + (i * T) % J, T), :] = y

    pending = []
    credit = [0.0]
    stretch = [STRETCH_A]

    def tick(cycles):
        if not pending:
            credit[0] = 0.0
            return
        credit[0] += cycles
        while pending and credit[0] >= stretch[0] * NQ * (pending[0][1] + 1):
            n, i = pending.pop(0)
            credit[0] -= stretch[0] * NQ * (i + 1) - 64
            conv_block(n, i)

    def drain():
        while pending:
            conv_block(*pending.pop(0))

    def front_k(n):
        sd = jnp.broadcast_to(_tile(vec(sd_ref), n), (8, LN))
        fk = _as_bf16(fk_ref[...])
        for m in range(NB):
            kf = _nt(fk, skb[n, :, pl.ds(m * T, T)])
            if m == 0:
                kf = jnp.concatenate(
                    [kf[8 * r:8 * r + 8] + sd if r % 2 == 0 else kf[8 * r:8 * r + 8]
                     for r in range(2 * NQ)], axis=0)
            gs[m * NT + n] = kf
            tick(64)

    def front_x(n):
        taps = sh_ref[...].astype(f32)
        fx = _as_bf16(fx_ref[...])
        a0, a1, a2, a3 = (jnp.broadcast_to(_tile(taps[i:i + 1], n), (T // 2, LN)) for i in range(4))
        for m in range(NB):
            base = KPAD // 2 + m * (T // 2)
            w0 = kw[n, pl.ds(base, T // 2), :]
            w1 = kw[n, pl.ds(base - 1, T // 2), :]
            w2 = kw[n, pl.ds(base - 2, T // 2), :]
            k0, k1, k2, k3, k4 = _hi(w0), _lo(w0), _hi(w1), _lo(w1), _hi(w2)
            vv = vw[n, pl.ds(m * (T // 2), T // 2), :]
            even = (a3 * k4 + a2 * k3 + a1 * k2 + a0 * k1) * _lo(vv)
            odd = (a3 * k3 + a2 * k2 + a1 * k1 + a0 * k0) * _hi(vv)
            parts = []
            for g in range(T // 16):
                parts += [even[8 * g:8 * g + 8], odd[8 * g:8 * g + 8]]
            xs[m * NT + n] = _nn(fx, jnp.concatenate(parts, axis=0).astype(bf16))
            tick(0)
        for i in range(NB):
            pending.append((n, i))

    zero = jnp.zeros((SEG, LN), f32)
    state = [(zero, zero) for _ in range(NT)]

    ub = {}

    def prep(c, chains=A_CHAINS):
        j0 = c * A_STEP

        def get(g):
            tiles = []
            for n in range(NT):
                parts = []
                for q in range(GROWS // 16):
                    row = j0 + g * GROWS // 8 + 2 * q
                    p = max(i for i, (r0, _) in enumerate(X_PARTS) if r0 <= row)
                    r0, r1 = X_PARTS[p]
                    w = xws[p][n, pl.ds((row - r0) // 2, SEG, stride=(r1 - r0) // 2), :]
                    parts += [_lo(w), _hi(w)]
                tiles.append(jnp.concatenate(parts, axis=0))
            return tiles

        def body(g, x0):
            u = _layernorm(x0)
            store_group(wp, j0, g, x0 + u * dsk)
            return u
        ub[c] = chained(chains, get, body, 8 * A_STEP).astype(bf16)

    def m_tiles(j0, nj, u, tiles, first=False):
        for n in tiles:
            b_tile(j0, nj, u, n, first)
            tick(20 * nj)

    def mm(c, tiles=range(NT), first=False):
        m_tiles(c * A_STEP, A_STEP, ub.pop(c) if NT - 1 in tiles else ub[c], tiles, first)

    wait(("x", 0), ("b", 0))
    start(("cv", 0))
    prep(0, WIDE)
    mm(0, range(0, 2), True)
    wait(("b", 1))
    start(("x", 1))
    prep(1)
    mm(0, range(2, NT), True)
    prep(2)
    mm(1)
    wait(("cv", 0), ("x", 1))
    start(("cv", 1), ("x", 2), ("cv", 2))
    front_k(0)
    prep(3)
    mm(2)
    front_x(0)
    wait(("cv", 1), ("x", 2))
    start(("x", 3))
    front_k(1)
    prep(4)
    mm(3)
    front_x(1)
    wait(("cv", 2))
    start(("cv", 3), "c")
    front_k(2)
    prep(5)
    mm(4)
    front_x(2)
    wait(("cv", 3), ("x", 3))
    start(("cv", 4), *[("bar", i) for i in range(NBAR)])
    front_k(3)
    prep(6)
    mm(5)
    prep(7)
    mm(6)
    front_x(3)
    wait(("cv", 4))
    front_k(4)
    mm(7)
    front_x(4)
    carry = segment_carry(state)
    h0 = fixup(0, B_STEP, carry)
    wait("c")

    stretch[0] = STRETCH_B
    for j0 in range(0, J, B_STEP):
        y = _nt(h0 if j0 == 0 else fixup(j0, B_STEP, carry), c_weights())
        rows = pl.ds(8 * j0, 8 * B_STEP)
        for n in range(NT):
            wp[n, rows, :] = wp[n, rows, :] + _tile(y, n)
        tick(100 * B_STEP)
    drain()

    def prep2(j0, chains):
        def body(g, x1):
            x2 = x1 + _layernorm(x1) * gate_group(j0, g)
            u = _layernorm(x2)
            store_group(wp, j0, g, x2 + u * dsk)
            return u
        return chained(chains, lambda g: row_group(wp, j0, g), body, 8 * C_STEP).astype(bf16)

    ub2 = prep2(0, C0_CHAINS)
    barrier()
    state[:] = [(zero, zero) for _ in range(NT)]
    for j0 in range(0, J, C_STEP):
        if j0 > 0:
            ub2 = prep2(j0, C_CHAINS)
        m_tiles(j0, C_STEP, ub2, range(NT))
    barrier()

    carry = segment_carry(state)
    anchors = {}
    j0 = 0
    for c, nj in enumerate(D_STEPS):
        for k, t in enumerate(anchors.pop(c - D_LAG, [])):
            carry[k % NT] = (carry[k % NT][0] + t, carry[k % NT][1])
        y = _nt(fixup(j0, nj, carry), c_weights())
        pitch = nj + 4

        def get(g):
            return [t + y[g * GROWS:(g + 1) * GROWS, n * LN:(n + 1) * LN]
                    for n, t in enumerate(row_group(wp, j0, g))]

        def body(g, x3):
            x4 = x3 + _layernorm(x3) * gate_group(j0, g)
            for n in range(NT):
                for j in range(GROWS // 8):
                    ob[c, n, pl.ds(g * GROWS // 8 + j, SEG, stride=pitch), :] = (
                        x4[8 * j:8 * j + 8, n * LN:(n + 1) * LN])
            return x4
        chained(D_CHAINS if c + D_LAG < len(D_STEPS) else WIDE, get, body, 8 * nj, True)
        anchors[c] = list(last_toks)
        for n in range(NT):
            for s in range(SEG):
                pltpu.make_async_copy(
                    ob.at[c, n, pl.ds(s * pitch, nj), :],
                    out_hbm.at[0, pl.ds(s * J + j0, nj), pl.ds(n * LN, LN)], osem).start()
        j0 += nj
    assert j0 == J and not plans and not started and bar_idx[0] == NBAR
    pltpu.make_async_copy(out_hbm, out_hbm, osem).wait()


@jax.jit
def pallas_interleave_layers__ssm_conv_s5__ssm_conv_h3__prompt_kernel(
    A_x: jax.Array,
    A_Lambda_re: jax.Array,
    A_Lambda_im: jax.Array,
    A_B_re: jax.Array,
    A_B_im: jax.Array,
    A_C_re: jax.Array,
    A_C_im: jax.Array,
    A_log_dt: jax.Array,
    A_Dskip: jax.Array,
    B_q: jax.Array,
    B_k: jax.Array,
    B_v: jax.Array,
    B_shift_k: jax.Array,
    B_ssm_k: jax.Array,
    B_ssm_D: jax.Array,
):
    del B_q
    bf, f32, u32 = jnp.bfloat16, jnp.float32, jnp.uint32
    n_sems = 13 + NBAR
    hbm = pl.BlockSpec(memory_space=pl.ANY)
    return pl.pallas_call(
        _kernel,
        out_shape=jax.ShapeDtypeStruct((1, S, D), f32),
        in_specs=[hbm] * 17,
        out_specs=hbm,
        scratch_shapes=[
            pltpu.VMEM((D,), bf), pltpu.VMEM((D,), bf), pltpu.VMEM((D,), bf), pltpu.VMEM((D,), bf),
            pltpu.VMEM((4, D), bf), pltpu.VMEM((D,), bf),
            pltpu.VMEM((T, T), u32), pltpu.VMEM((T, T), u32), pltpu.VMEM((T // 2 + 8, 2 * T), u32),
            *[pltpu.VMEM((NT, SEG * (r1 - r0), LN), bf) for r0, r1 in X_PARTS],
            pltpu.VMEM((2, D, D), bf),
            pltpu.VMEM((2, D // 2, D), u32),
            pltpu.VMEM((2, NT, D, LN), bf),
            pltpu.VMEM((NT, KPAD + S, LN), bf),
            pltpu.VMEM((NT, S, LN), bf),
            pltpu.VMEM((NT, LN, S), bf),
            pltpu.VMEM((NB * NT, 2 * T, LN), f32),
            pltpu.VMEM((NB * NT, 2 * T, LN), f32),
            pltpu.VMEM((NB * NT, 2 * T, LN), f32),
            pltpu.VMEM((NT, SEG * PF, LN), f32),
            pltpu.VMEM((NT, S, LN), f32),
            pltpu.VMEM((NT, S, LN), f32),
            pltpu.VMEM((NT, S, LN), f32),
            pltpu.VMEM((len(D_STEPS), NT, SEG * (max(D_STEPS) + 4), LN), f32),
            pltpu.VMEM((NBAR, 16, LN), bf),
            pltpu.SemaphoreType.DMA((n_sems,)),
            pltpu.SemaphoreType.DMA(()),
        ],
        compiler_params=pltpu.CompilerParams(
            vmem_limit_bytes=112 * 1024 * 1024,
            flags={"XLA_TPU_EVENLY_DISTRIBUTE_CRITICAL_NODES": True}),
    )(A_Lambda_re, A_Lambda_im, A_log_dt, A_Dskip, B_shift_k.T, B_ssm_D, _FK, _FX, _INV,
      A_x, A_B_re, A_B_im, A_C_re, A_C_im, B_k, B_v, B_ssm_k)
```
